```python
import jax
import jax.numpy as jnp

def _softmax(x, axis=-1):
    return jax.nn.softmax(x, axis=axis)

def _gelu(x):
    return jax.nn.gelu(x, approximate=True)

def _silu(x):
    return jax.nn.silu(x)

def _sigmoid(x):
    return jax.nn.sigmoid(x)

def _layernorm(x, axis=-1, eps=1e-05):
    m = jnp.mean(x, axis=axis, keepdims=True)
    v = jnp.var(x, axis=axis, keepdims=True)
    return (x - m) / jnp.sqrt(v + eps)

def _scatter_add(tgt, idx, src, axis=0):
    return tgt.at[idx].add(src)

def _segment_sum(src, seg, n):
    return jax.ops.segment_sum(src, seg, n)

class _Rng:

    def __init__(self, key):
        self._k = key

    def _next(self):
        self._k, sub = jax.random.split(self._k)
        return sub

    def normal(self, shape):
        return jax.random.normal(self._next(), shape, dtype=jnp.bfloat16)

    def randint(self, lo, hi, shape):
        return jax.random.randint(self._next(), shape, lo, hi, dtype=jnp.int32)

    def uniform(self, shape, lo=0.0, hi=1.0):
        return jax.random.uniform(self._next(), shape, jnp.bfloat16, lo, hi)

    def permutation(self, n):
        return jax.random.permutation(self._next(), n)
kernel_name = 'interleave_layers__memory_aug_recurrent_mem_tr__glu_gated_geglu__prompt'

def setup_inputs():
    _rng = _Rng(jax.random.key(int.from_bytes(__import__("os").urandom(4), "little")))
    _w = lambda a: (lambda t: t.astype(jnp.bfloat16) if jnp.issubdtype(t.dtype, jnp.floating) else t)(jnp.asarray(a))

    def _A_setup():
        B, S, Dm = (1, 2048, 1024)
        H, Dh = (32, 128)
        M, seg = (8, 32)
        seg = min(seg, S)
        S = S // seg * seg
        return {'x': _w((lambda *s: _rng.normal(s) * 0.05)(B, S, Dm)), 'mem0': _w((lambda *s: _rng.normal(s) * 0.05)(B, M, Dm)), 'Wq': _w((lambda *s: _rng.normal(s) * 0.05)(Dm, H, Dh) * Dm ** (-0.5)), 'Wk': _w((lambda *s: _rng.normal(s) * 0.05)(Dm, H, Dh) * Dm ** (-0.5)), 'Wv': _w((lambda *s: _rng.normal(s) * 0.05)(Dm, H, Dh) * Dm ** (-0.5)), 'Wo': _w((lambda *s: _rng.normal(s) * 0.05)(H, Dh, Dm) * (H * Dh) ** (-0.5)), 'seg_len': seg}
    _A_in = _A_setup()

    def _B_setup():
        B, S, Dm, Df = (1, 2048, 1024, 3584)
        return {'x': _w((lambda *s: _rng.normal(s) * 0.05)(B, S, Dm)), 'w_gate': _w((lambda *s: _rng.normal(s) * 0.05)(Dm, Df) * Dm ** (-0.5)), 'w_up': _w((lambda *s: _rng.normal(s) * 0.05)(Dm, Df) * Dm ** (-0.5)), 'w_down': _w((lambda *s: _rng.normal(s) * 0.05)(Df, Dm) * Df ** (-0.5))}
    _B_in = _B_setup()
    return {'A_x': _A_in['x'], 'A_mem0': _A_in['mem0'], 'A_Wq': _A_in['Wq'], 'A_Wk': _A_in['Wk'], 'A_Wv': _A_in['Wv'], 'A_Wo': _A_in['Wo'], 'A_seg_len': _A_in['seg_len'], 'B_x': _B_in['x'], 'B_w_gate': _B_in['w_gate'], 'B_w_up': _B_in['w_up'], 'B_w_down': _B_in['w_down']}

def reference(A_x, A_mem0, A_Wq, A_Wk, A_Wv, A_Wo, A_seg_len, B_x, B_w_gate, B_w_up, B_w_down):

    def _A_ref(x, mem0, Wq, Wk, Wv, Wo, seg_len):
        B, S, Dm = x.shape
        H, Dh = (Wq.shape[1], Wq.shape[2])
        M = mem0.shape[1]
        scale = Dh ** (-0.5)
        n_seg = S // seg_len
        L = M + seg_len
        idx = jnp.arange(L)
        mask = (idx[:, None] < M) | (idx[:, None] >= idx[None, :])
        mem = mem0
        outs = []
        for s in range(n_seg):
            xs = x[:, s * seg_len:(s + 1) * seg_len, :].copy()
            h = jnp.concatenate([mem, xs], axis=1)
            q = jnp.einsum('btd,dhe->bhte', h, Wq)
            k = jnp.einsum('btd,dhe->bhte', h, Wk)
            v = jnp.einsum('btd,dhe->bhte', h, Wv)
            scores = jnp.einsum('bhqe,bhke->bhqk', q, k) * scale
            scores = jnp.where(mask[None, None], scores, -1000000000.0)
            p = _softmax(scores, axis=-1)
            o = jnp.einsum('bhqk,bhke->bhqe', p, v)
            o = jnp.einsum('bhte,hed->btd', o, Wo)
            mem = o[:, :M, :].copy()
            outs.append(o[:, M:, :])
        return jnp.concatenate(outs, axis=1)

    def _B_ref(x, w_gate, w_up, w_down):
        g = jnp.einsum('bsd,df->bsf', x, w_gate)
        u = jnp.einsum('bsd,df->bsf', x, w_up)
        h = _gelu(g) * u
        return jnp.einsum('bsf,fd->bsd', h, w_down)
    x = A_x
    x = x + _A_ref(_layernorm(x, axis=-1), A_mem0, A_Wq, A_Wk, A_Wv, A_Wo, A_seg_len)
    x = x + _B_ref(_layernorm(x, axis=-1), B_w_gate, B_w_up, B_w_down)
    x = x + _A_ref(_layernorm(x, axis=-1), A_mem0, A_Wq, A_Wk, A_Wv, A_Wo, A_seg_len)
    x = x + _B_ref(_layernorm(x, axis=-1), B_w_gate, B_w_up, B_w_down)
    return x
```

```python
import functools
import jax
import jax.numpy as jnp
import numpy as np
from jax import lax
from jax.experimental import pallas as pl
from jax.experimental.pallas import tpu as pltpu

BF = jnp.bfloat16
F32 = jnp.float32
U32 = jnp.uint32
NT = (((1,), (1,)), ((), ()))
LANES = 128


def _ln(x):
    m = jnp.mean(x, axis=-1, keepdims=True)
    c = x - m
    v = jnp.mean(c * c, axis=-1, keepdims=True)
    return c * lax.rsqrt(v + 1e-5)


def _gelu(g):
    c0 = float(np.sqrt(2.0 / np.pi))
    return 0.5 * g * (1.0 + jnp.tanh(g * (c0 + (c0 * 0.044715) * (g * g))))


def _dot(a, b):
    return jnp.dot(a, b, preferred_element_type=F32)


def build(S, D, H, E, M, SEG, DF, HG=2, FC=4, OG=4, flags=None, NCH=8, L=(1, 2, 3), order="pqwv", NQ=4,
          DP=((0, "q", 6), (1, "q", 12), (1, "v", 18)), LP=(1, 2, 3), orderP="pqwv", LS=(1, 2, 3), orderS="pqwv",
          NP=7, NST=None, LA=3, VH=8, QI=2, QH=4, RK=2, TD=(0, 5, 6, 8), SL=False, LAG=2, WIDE=(), RF=False, SUB=16, PP=2, WO_D=0, FF_AT=4, X_AT=6, UN=1, NPL=None, NS1=None, NS2=None):
    NS1 = LAG if NS1 is None else NS1
    NST = S // SEG - LAG if NST is None else NST
    assert all(t < LA + (QI - 1) * NCH for t in TD) and LA + QI * NCH <= 3 * NCH
    NS2 = LAG if NS2 is None else NS2
    NPL = NP if NPL is None else NPL
    NS = S // SEG
    R2, R1 = 2 * M + 2 * SEG, 2 * M + SEG
    G = H // HG
    ND = D // LANES
    NF = DF // LANES
    scale = float(E ** -0.5)
    CH = D // NCH
    HC = H // NCH
    X0 = LAG + NP + 1

    def seg(s, n=1):
        return pl.ds(pl.multiple_of(s * SEG, SEG), n * SEG)

    def kern(x_hbm, mem_ref, wq_hbm, wk_hbm, wv_hbm, wo_hbm, wg_hbm, wu_hbm, wd_hbm, o_hbm,
             x_v, stage, wq, wk, wv, wo, wg, wu, wd, h_ref, qkv_ref, o_ref, acc_ref, x2_v, xr_ref, hf_ref, a_ref, yacc_ref, y_v,
             hp_ref, hc_ref, pre_ref, sems, wsems, tsems):
        wqkv = (wq, wk, wv)
        x_cp0 = pltpu.make_async_copy(x_hbm.at[0:X0 * SEG, :], x_v.at[0:X0 * SEG, :], sems.at[0])
        x_cp1 = pltpu.make_async_copy(x_hbm.at[X0 * SEG:S, :], x_v.at[X0 * SEG:S, :], sems.at[2])
        st_cps = [pltpu.make_async_copy(w.at[pl.ds(c * CH * H, CH * H), :], stage.at[i * NCH + c], wsems.at[i * NCH + c])
                  for i, w in enumerate((wq_hbm, wk_hbm, wv_hbm)) for c in range(NCH)]
        t_cps = []
        for i, (src, dst, n) in enumerate(((wo_hbm, wo, ND), (wg_hbm, wg, NF), (wu_hbm, wu, NF), (wd_hbm, wd, ND))):
            if i in WIDE:
                t_cps.append([pltpu.make_async_copy(src, dst, tsems.at[i])])
            else:
                t_cps.append([pltpu.make_async_copy(src.at[:, j * LANES:(j + 1) * LANES], dst.at[j], tsems.at[i]) for j in range(n)])
        x_cp0.start()
        for c in st_cps[0:LA]:
            c.start()

        def static_loop(lo, hi):
            def run(f):
                for c in range(lo, hi):
                    f(c)
            return run

        def start_chunk(i):
            if isinstance(i, int):
                if i < 3 * NCH:
                    st_cps[i].start()
                elif i == 3 * NCH + WO_D:
                    for c in t_cps[0]:
                        c.start()
                return
            for n, w in enumerate((wq_hbm, wk_hbm, wv_hbm)):
                @pl.when(i // NCH == n)
                def _():
                    src = w.at[pl.ds(pl.multiple_of((i - n * NCH) * (CH * H), CH * H), CH * H), :]
                    pltpu.make_async_copy(src, stage.at[i], wsems.at[i]).start()

            for n in range(4):
                @pl.when(i == 3 * NCH + TD[n])
                def _():
                    start_all(t_cps[n])

        def relayout(n, c, lo, hi):
            for b in range(lo, hi):
                x = pltpu.bitcast(stage[n * NCH + c, b * SUB * H:(b + 1) * SUB * H, :], U32).reshape(SUB // 2, 2, H // 2, E)
                ev, od = x[:, 0], x[:, 1]
                lo_h = jnp.swapaxes((ev & U32(0xFFFF)) | (od << 16), 0, 1)
                hi_h = jnp.swapaxes((ev >> 16) | (od & U32(0xFFFF0000)), 0, 1)
                r0 = c * (CH // 2) + b * (SUB // 2)
                r = pl.ds(r0 if isinstance(c, int) else pl.multiple_of(r0, SUB // 2), SUB // 2)
                for hp in range(H // 2):
                    wqkv[n][2 * hp, r, :] = lo_h[hp]
                    wqkv[n][2 * hp + 1, r, :] = hi_h[hp]

        def arrive(i):
            pltpu.make_async_copy(stage.at[i], stage.at[i], wsems.at[i]).wait()
            start_chunk(i + LA)

        def preproj(n, h0, nh):
            w = jnp.concatenate([pltpu.bitcast(wqkv[n][h0 + j], BF) for j in range(nh)], axis=1)
            r = _dot(hp_ref[...], w).astype(BF)
            for j in range(nh):
                pre_ref[n * H + h0 + j] = r[:, j * E:(j + 1) * E]

        def start_all(cps):
            for c in cps:
                c.start()

        NB = CH // SUB

        PR = NP * SEG
        HB = D // E
        x_cp0.wait()
        for s in range(NP):
            xn = _ln(x_v[(LAG + s) * SEG:(LAG + s + 1) * SEG, :].astype(F32)).astype(BF)
            hp_ref[s * SEG:(s + 1) * SEG, :] = xn
            for c in range(NCH):
                hc_ref[c, s * SEG:(s + 1) * SEG, :] = xn[:, c * CH:(c + 1) * CH]
        x2_v[0:(H // HB) * PR, :] = jnp.zeros(((H // HB) * PR, D), F32)

        def arrive2(i, nxt):
            pltpu.make_async_copy(stage.at[i], stage.at[i], wsems.at[i]).wait()
            for n in nxt:
                start_chunk(n)

        @pl.loop(0, NCH)
        def _(c):
            arrive2(c, [LA + QI * c + u for u in range(QI)])
            relayout(0, c, 0, NB)
            r = pl.ds(pl.multiple_of(c * (CH // 2), CH // 2), CH // 2)
            for j in range(H // HB):
                for j2 in range(0, HB, QH):
                    w = jnp.concatenate([pltpu.bitcast(wq[j * HB + j2 + u, r, :], BF) for u in range(QH)], axis=1)
                    x2_v[j * PR:(j + 1) * PR, j2 * E:(j2 + QH) * E] += _dot(hc_ref[c], w)
        for h in range(H):
            pre_ref[h] = x2_v[(h // HB) * PR:(h // HB + 1) * PR, (h % HB) * E:(h % HB + 1) * E].astype(BF)
        I1 = LA + QI * NCH

        @pl.loop(0, NCH // RK)
        def _(c):
            for u in range(RK):
                arrive2(NCH + c * RK + u, [I1 + c * RK + u])
                relayout(1, c * RK + u, 0, NB)

        @pl.loop(0, NCH)
        def _(c):
            arrive2(2 * NCH + c, [I1 + NCH + c])
            relayout(2, c, 0, NB)
            preproj(1, c * HC, HC)

        @pl.loop(0, H // VH)
        def _(c):
            preproj(2, c * VH, VH)

        def proj(g, R, pre):
            heads = [(i, g * HG + j) for i in range(3) for j in range(HG)]
            w = jnp.concatenate([pltpu.bitcast(wqkv[i][n], BF) for i, n in heads], axis=1)
            RP = R if pre is None else R1
            qkv_ref[g % NQ, 0:RP, :] = _dot(h_ref[0:RP, :], w).astype(BF)
            if pre is not None:
                for j, (i, n) in enumerate(heads):
                    qkv_ref[g % NQ, R1:R2, j * E:(j + 1) * E] = pre_ref[i * H + n, pre, :]

        def qk(g, R):
            ri = lax.broadcasted_iota(jnp.int32, (R, R), 0)
            ci = lax.broadcasted_iota(jnp.int32, (R, R), 1)
            lay = lambda i: jnp.where(i < 2 * M, (i >= M).astype(jnp.int32), (i >= R1).astype(jnp.int32))
            same = lay(ri) == lay(ci)
            valid = same & ((ri < 2 * M) | (ri >= ci))
            fill = jnp.where(same, -1e9, -jnp.inf).astype(F32)
            slot = g % NQ
            res = []
            for j in range(HG):
                q = qkv_ref[slot, 0:R, j * E:(j + 1) * E]
                k = qkv_ref[slot, 0:R, (HG + j) * E:(HG + j + 1) * E]
                s = lax.dot_general(q, k, NT, preferred_element_type=F32) * scale
                s = jnp.where(valid, s, fill)
                p = jnp.exp(s - jnp.max(s, axis=-1, keepdims=True))
                res.append((p.astype(BF), 1.0 / jnp.sum(p, axis=-1, keepdims=True)))
            return res

        def pv(g, R, res):
            for j in range(HG):
                v = qkv_ref[g % NQ, 0:R, (2 * HG + j) * E:(2 * HG + j + 1) * E]
                p, r = res[j]
                o_ref[g * HG + j, 0:R, :] = (_dot(p, v) * r).astype(BF)

        def cols(i, ref, rows, lo, hi):
            if i in WIDE:
                return [ref[rows, lo * LANES:hi * LANES]]
            return [ref[j, rows, :] for j in range(lo, hi)]

        def wout(c, R):
            o = jnp.concatenate([o_ref[c * OG + j, 0:R, :] for j in range(OG)], axis=1)
            w = jnp.concatenate(cols(0, wo, slice(c * OG * E, (c + 1) * OG * E), 0, ND), axis=1)
            r = _dot(o, w)
            if c > 0:
                r = r + acc_ref[0:R, :]
            if c == H // OG - 1:
                return r
            acc_ref[0:R, :] = r

        def attention(R, L, order, fillers=(), pre=None):
            ps = {}
            nxt = 0
            fillers = dict(fillers)
            for g in range(G + max(L) + 1):
                for op in order:
                    if op == "p" and g < G:
                        proj(g, R, pre)
                    if op == "q" and 0 <= g - L[0] < G:
                        ps[g - L[0]] = qk(g - L[0], R)
                    if op == "v" and 0 <= g - L[1] < G:
                        pv(g - L[1], R, ps.pop(g - L[1]))
                    if op == "w":
                        while nxt < H // OG and (nxt + 1) * OG <= (g - L[2] + 1) * HG:
                            out = wout(nxt, R)
                            nxt += 1
                    if (g - G, op) in fillers:
                        fillers.pop((g - G, op))()
            assert nxt == H // OG and not fillers
            return out

        def gate_up():
            for c in range(NF // FC):
                w = jnp.concatenate(cols(1, wg, slice(None), c * FC, (c + 1) * FC) + cols(2, wu, slice(None), c * FC, (c + 1) * FC), axis=1)
                gu = _dot(hf_ref[...], w)
                a_ref[:, c * FC * LANES:(c + 1) * FC * LANES] = (_gelu(gu[:, :FC * LANES]) * gu[:, FC * LANES:]).astype(BF)

        def down(lo, hi):
            rs = slice(lo * LANES, hi * LANES)
            return _dot(a_ref[:, rs], jnp.concatenate(cols(3, wd, rs, 0, ND), axis=1))

        def set_f(half, xr):
            xr_ref[half * SEG:(half + 1) * SEG, :] = xr
            hf_ref[half * SEG:(half + 1) * SEG, :] = _ln(xr).astype(BF)

        def out_copy(s):
            return pltpu.make_async_copy(y_v.at[seg(s), :], o_hbm.at[seg(s), :], sems.at[1])

        mem0 = mem_ref[...].astype(F32)
        h_ref[0:2 * M, :] = jnp.concatenate([mem0, mem0], axis=0).astype(BF)
        h_ref[2 * M:R1, :] = _ln(x_v[0:SEG, :].astype(F32)).astype(BF)
        for c in t_cps[0]:
            c.wait()

        def solo1(s, carry):
            out = attention(R1, LS, orderS)
            x2_v[seg(s), :] = x_v[seg(s), :].astype(F32) + out[2 * M:, :]
            h_ref[0:2 * M, :] = out[0:2 * M, :].astype(BF)
            h_ref[2 * M:R1, :] = _ln(x_v[seg(s + 1), :].astype(F32)).astype(BF)
            return carry
        lax.fori_loop(0, NS1, solo1, 0)
        for c in t_cps[1] + t_cps[2]:
            c.wait()
        set_f(0, x2_v[0:SEG, :])
        set_f(1, x2_v[SEG:2 * SEG, :])
        gate_up()
        for c in t_cps[3]:
            c.wait()
        x_cp1.start()
        x2_v[0:2 * SEG, :] = xr_ref[...] + down(0, NF)
        mem1 = h_ref[0:M, :].astype(F32)
        h_ref[0:2 * M, :] = jnp.concatenate([mem0, mem1], axis=0).astype(BF)

        def finish_attention(t, out):
            set_f(0, x2_v[seg(t - LAG), :] + out[2 * M:R1, :])
            set_f(1, x_v[seg(t), :].astype(F32) + out[R1:, :])
            h_ref[0:2 * M, :] = out[0:2 * M, :].astype(BF)

        T0 = LAG
        if LAG == 4:
            set_f(0, x2_v[2 * SEG:3 * SEG, :])
            set_f(1, x2_v[3 * SEG:4 * SEG, :])
        else:
            h_ref[2 * M:R1, :] = _ln(x2_v[0:SEG, :]).astype(BF)
            finish_attention(LAG, attention(R2, LP, orderP, pre=slice(0, SEG)))
            T0 = LAG + 1

        def steady(t, carry, pre):
            @pl.when(t >= LAG + 2)
            def _():
                out_copy(t - LAG - 2).start()
            h_ref[2 * M:R1, :] = _ln(x2_v[seg(t - LAG), :]).astype(BF)
            gate_up()

            def part(lo, hi):
                def f():
                    yacc_ref[...] = (xr_ref[...] if lo == 0 else yacc_ref[...]) + down(lo, hi)
                return f
            cuts = [0] + [c for _, _, c in DP]
            fillers = {(g, op): part(cuts[i], c) for i, (g, op, c) in enumerate(DP)}
            if pre:
                out = attention(R2, LP, orderP, fillers, seg(t - LAG))
            else:
                out = attention(R2, L, order, fillers)
            finish_attention(t, out)
            h_ref[R1:R2, :] = _ln(x_v[seg(jnp.minimum(t + 1, NS - 1)), :].astype(F32)).astype(BF)
            y = yacc_ref[...] + down(cuts[-1], NF)
            x2_v[seg(t - 1), :] = y[SEG:]
            if LAG == 4:
                x2_v[seg(jnp.where(t == LAG, LAG - 2, NS)), :] = y[0:SEG]
            y_v[seg(jnp.maximum(t - 1 - LAG, 0)), :] = y[0:SEG].astype(BF)
            return carry
        lax.fori_loop(T0, LAG + NPL, functools.partial(steady, pre=True), 0)
        x_cp1.wait()
        lax.fori_loop(LAG + NP, LAG + NST, functools.partial(steady, pre=False), 0, unroll=UN)

        out_copy(NS - LAG - 2).start()
        gate_up()
        y = xr_ref[...] + down(0, NF)
        x2_v[(NS - 1) * SEG:NS * SEG, :] = y[SEG:]
        y_v[(NS - 1 - LAG) * SEG:(NS - LAG) * SEG, :] = y[0:SEG].astype(BF)
        out_copy(NS - LAG - 1).start()

        def solo2(s, carry):
            out = attention(R1, LS, orderS)
            x2_v[seg(s), :] = x2_v[seg(s), :] + out[2 * M:, :]
            h_ref[0:2 * M, :] = out[0:2 * M, :].astype(BF)
            h_ref[2 * M:R1, :] = _ln(x2_v[seg(jnp.minimum(s + 1, NS - 1)), :]).astype(BF)
            return carry
        h_ref[2 * M:R1, :] = _ln(x2_v[(NS - LAG) * SEG:(NS - LAG + 1) * SEG, :]).astype(BF)
        lax.fori_loop(NS - LAG, NS - LAG + NS2, solo2, 0)

        def last_f(i, carry):
            s = NS - LAG + 2 * i
            set_f(0, x2_v[seg(s), :])
            set_f(1, x2_v[seg(s + 1), :])
            gate_up()
            y_v[seg(s, 2), :] = (xr_ref[...] + down(0, NF)).astype(BF)
            out_copy(s).start()
            out_copy(s + 1).start()
            return carry
        lax.fori_loop(0, LAG // 2, last_f, 0)
        ts = list(range(T0, LAG + NPL)) + list(range(LAG + NP, LAG + NST))
        nw = (sum(t >= LAG + 2 for t in ts) + 2 + LAG) * SEG
        pltpu.make_async_copy(y_v.at[0:nw, :], o_hbm.at[0:nw, :], sems.at[1]).wait()

    any_spec = pl.BlockSpec(memory_space=pl.ANY)
    return pl.pallas_call(
        kern,
        out_shape=jax.ShapeDtypeStruct((S, D), BF),
        in_specs=[any_spec, pl.BlockSpec(memory_space=pltpu.VMEM)] + [any_spec] * 7,
        out_specs=any_spec,
        scratch_shapes=[
            pltpu.VMEM((S, D), BF), pltpu.VMEM((3 * NCH, CH * H, E), BF), pltpu.VMEM((H, D // 2, E), U32), pltpu.VMEM((H, D // 2, E), U32), pltpu.VMEM((H, D // 2, E), U32),
            *[pltpu.VMEM((r, c * LANES) if i in WIDE else (c, r, LANES), BF)
              for i, (r, c) in enumerate(((H * E, ND), (D, NF), (D, NF), (DF, ND)))],
            pltpu.VMEM((R2, D), BF), pltpu.VMEM((NQ, R2, 3 * HG * E), BF), pltpu.VMEM((H, R2, E), BF), pltpu.VMEM((R2, D), F32),
            pltpu.VMEM((S + SEG, D), F32), pltpu.VMEM((2 * SEG, D), F32), pltpu.VMEM((2 * SEG, D), BF),
            pltpu.VMEM((2 * SEG, DF), BF), pltpu.VMEM((2 * SEG, D), F32), pltpu.VMEM((S, D), BF),
            pltpu.VMEM((NP * SEG, D), BF), pltpu.VMEM((NCH, NP * SEG, CH), BF), pltpu.VMEM((3 * H, NP * SEG, E), BF),
            pltpu.SemaphoreType.DMA((3,)), pltpu.SemaphoreType.DMA((3 * NCH,)), pltpu.SemaphoreType.DMA((4,)),
        ],
        compiler_params=pltpu.CompilerParams(vmem_limit_bytes=124 * 2**20, flags=flags),
    )


@functools.partial(jax.jit, static_argnames=("A_seg_len",))
def pallas_interleave_layers__memory_aug_recurrent_mem_tr__glu_gated_geglu__prompt_kernel(
    A_x, A_mem0, A_Wq, A_Wk, A_Wv, A_Wo, A_seg_len, B_x, B_w_gate, B_w_up, B_w_down
):
    del B_x
    _, S, D = A_x.shape
    _, H, E = A_Wq.shape
    M = A_mem0.shape[1]
    y = build(S, D, H, E, M, int(A_seg_len), B_w_gate.shape[1], NP=11, LA=2, TD=(0, 4, 6, 8))(
        A_x.reshape(S, D), A_mem0.reshape(M, D), A_Wq.reshape(D * H, E), A_Wk.reshape(D * H, E),
        A_Wv.reshape(D * H, E), A_Wo.reshape(H * E, D), B_w_gate, B_w_up, B_w_down)
    return y.reshape(1, S, D)
```

```python
import functools
import jax
import jax.numpy as jnp
import numpy as np
from jax import lax
from jax.experimental import pallas as pl
from jax.experimental.pallas import tpu as pltpu

BF = jnp.bfloat16
F32 = jnp.float32
U32 = jnp.uint32
NT = (((1,), (1,)), ((), ()))
LANES = 128


def _ln(x):
    m = jnp.mean(x, axis=-1, keepdims=True)
    c = x - m
    v = jnp.mean(c * c, axis=-1, keepdims=True)
    return c * lax.rsqrt(v + 1e-5)


def _gelu(g):
    c0 = float(np.sqrt(2.0 / np.pi))
    return 0.5 * g * (1.0 + jnp.tanh(g * (c0 + (c0 * 0.044715) * (g * g))))


def _dot(a, b):
    return jnp.dot(a, b, preferred_element_type=F32)


def build(S, D, H, E, M, SEG, DF, HG=2, FC=4, OG=4, flags=None, NCH=8, L=(1, 2, 3), order="pqwv", NQ=4,
          DP=((0, "q", 6), (1, "q", 12), (1, "v", 18)), LP=(1, 2, 3), orderP="pqwv", LS=(1, 2, 3), orderS="pqwv",
          NP=14, NST=None, LA=2, VH=8, QI=2, QH=4, RK=2, TD=(0, 4, 6, 8), SL=False, LAG=2, WIDE=(), RF=False, SUB=16, PP=2, WO_D=0, FF_AT=4, X_AT=6, UN=1, USEPRE=True, PEEL=0, NPL=None, NS1=None, NS2=None):
    NS1 = LAG if NS1 is None else NS1
    NST = S // SEG - LAG if NST is None else NST
    assert LAG == 2
    assert all(t < LA + (QI - 1) * NCH for t in TD) and LA + QI * NCH <= 3 * NCH
    NS2 = LAG if NS2 is None else NS2
    NPL = NP if NPL is None else NPL
    NS = S // SEG
    R2, R1 = 2 * M + 2 * SEG, 2 * M + SEG
    G = H // HG
    ND = D // LANES
    NF = DF // LANES
    scale = float(E ** -0.5)
    CH = D // NCH
    HC = H // NCH
    X0 = LAG + NP + 1

    def seg(s, n=1):
        return pl.ds(pl.multiple_of(s * SEG, SEG), n * SEG)

    def kern(x_hbm, mem_ref, wq_hbm, wk_hbm, wv_hbm, wo_hbm, wg_hbm, wu_hbm, wd_hbm, o_hbm,
             x_v, stage, wqkv, wo, wg, wu, wd, h_ref, qkv_ref, o_ref, acc_ref, x2_v, xr_ref, hf_ref, a_ref, yacc_ref, y_v,
             hc_ref, pre_ref, sems, wsems, tsems):
        x_cp0 = pltpu.make_async_copy(x_hbm.at[0:X0 * SEG, :], x_v.at[0:X0 * SEG, :], sems.at[0])
        x_cp1 = pltpu.make_async_copy(x_hbm.at[X0 * SEG:S, :], x_v.at[X0 * SEG:S, :], sems.at[2])
        st_cps = [pltpu.make_async_copy(wq_hbm.at[pl.ds(c * CH * H, CH * H), :], stage.at[c], wsems.at[c]) for c in range(LA)]
        t_cps = []
        for i, (src, dst, n) in enumerate(((wo_hbm, wo, ND), (wg_hbm, wg, NF), (wu_hbm, wu, NF), (wd_hbm, wd, ND))):
            if i in WIDE:
                t_cps.append([pltpu.make_async_copy(src, dst, tsems.at[i])])
            else:
                t_cps.append([pltpu.make_async_copy(src.at[:, j * LANES:(j + 1) * LANES], dst.at[j], tsems.at[i]) for j in range(n)])
        x_cp0.start()
        for c in st_cps[0:LA]:
            c.start()

        def static_loop(lo, hi):
            def run(f):
                for c in range(lo, hi):
                    f(c)
            return run

        def start_chunk(i):
            for n, w in enumerate((wq_hbm, wk_hbm, wv_hbm)):
                @pl.when(i // NCH == n)
                def _():
                    src = w.at[pl.ds(pl.multiple_of((i - n * NCH) * (CH * H), CH * H), CH * H), :]
                    pltpu.make_async_copy(src, stage.at[i], wsems.at[i]).start()

            for n in range(4):
                @pl.when(i == 3 * NCH + TD[n])
                def _():
                    start_all(t_cps[n])

        def relayout(n, c, lo, hi):
            for b in range(lo, hi):
                x = pltpu.bitcast(stage[n * NCH + c, b * SUB * H:(b + 1) * SUB * H, :], U32).reshape(SUB // 2, 2, H // 2, E)
                ev, od = x[:, 0], x[:, 1]
                lo_h = jnp.swapaxes((ev & U32(0xFFFF)) | (od << 16), 0, 1)
                hi_h = jnp.swapaxes((ev >> 16) | (od & U32(0xFFFF0000)), 0, 1)
                r0 = c * (CH // 2) + b * (SUB // 2)
                r = pl.ds(pl.multiple_of(r0, SUB // 2), SUB // 2)
                for hp in range(H // 2):
                    wqkv[n * H + 2 * hp, r, :] = lo_h[hp]
                    wqkv[n * H + 2 * hp + 1, r, :] = hi_h[hp]

        def start_all(cps):
            for c in cps:
                c.start()

        NB = CH // SUB

        PR = NP * SEG
        HB = D // E
        x_cp0.wait()
        for s in range(NP):
            xn = _ln(x_v[(LAG + s) * SEG:(LAG + s + 1) * SEG, :].astype(F32)).astype(BF)
            for c in range(NCH):
                hc_ref[c, s * SEG:(s + 1) * SEG, :] = xn[:, c * CH:(c + 1) * CH]

        def pre_chunk(n, c, first=False, last=False):
            i = n * NCH + c
            pltpu.make_async_copy(stage.at[i], stage.at[i], wsems.at[i]).wait()
            i1 = LA + i + (QI - 1) * jnp.where(n == 0, c, NCH - 1)

            @pl.loop(i1, i1 + jnp.where(n == 0, QI, 1))
            def _(j):
                start_chunk(j + jnp.where(n == 0, 0, QI - 1))
            relayout(n, c, 0, NB)
            r = pl.ds(pl.multiple_of(c * (CH // 2), CH // 2), CH // 2)
            for h0 in range(0, H, QH):
                w = jnp.concatenate([pltpu.bitcast(wqkv[n * H + h0 + u, r, :], BF) for u in range(QH)], axis=1)
                blk = (slice((h0 // HB) * PR, (h0 // HB + 1) * PR), slice((h0 % HB) * E, (h0 % HB + QH) * E))
                res = _dot(hc_ref[c], w)
                if not first:
                    res = res + x2_v[blk]
                if last:
                    for u in range(QH):
                        pre_ref[n * H + h0 + u] = res[:, u * E:(u + 1) * E].astype(BF)
                else:
                    x2_v[blk] = res

        @pl.loop(0, 3)
        def _(n):
            pre_chunk(n, 0, first=True)
            pl.loop(1, NCH - 1)(functools.partial(pre_chunk, n))
            pre_chunk(n, NCH - 1, last=True)

        def proj(g, R, pre):
            heads = [(i, g * HG + j) for i in range(3) for j in range(HG)]
            w = jnp.concatenate([pltpu.bitcast(wqkv[i * H + n], BF) for i, n in heads], axis=1)
            RP = R if pre is None else R1
            qkv_ref[g % NQ, 0:RP, :] = _dot(h_ref[0:RP, :], w).astype(BF)
            if pre is not None:
                for j, (i, n) in enumerate(heads):
                    qkv_ref[g % NQ, R1:R2, j * E:(j + 1) * E] = pre_ref[i * H + n, pre, :]

        def qk(g, R):
            ri = lax.broadcasted_iota(jnp.int32, (R, R), 0)
            ci = lax.broadcasted_iota(jnp.int32, (R, R), 1)
            lay = lambda i: jnp.where(i < 2 * M, (i >= M).astype(jnp.int32), (i >= R1).astype(jnp.int32))
            same = lay(ri) == lay(ci)
            valid = same & ((ri < 2 * M) | (ri >= ci))
            fill = jnp.where(same, -1e9, -jnp.inf).astype(F32)
            slot = g % NQ
            res = []
            for j in range(HG):
                q = qkv_ref[slot, 0:R, j * E:(j + 1) * E]
                k = qkv_ref[slot, 0:R, (HG + j) * E:(HG + j + 1) * E]
                s = lax.dot_general(q, k, NT, preferred_element_type=F32) * scale
                s = jnp.where(valid, s, fill)
                p = jnp.exp(s - jnp.max(s, axis=-1, keepdims=True))
                res.append((p.astype(BF), 1.0 / jnp.sum(p, axis=-1, keepdims=True)))
            return res

        def pv(g, R, res):
            for j in range(HG):
                v = qkv_ref[g % NQ, 0:R, (2 * HG + j) * E:(2 * HG + j + 1) * E]
                p, r = res[j]
                o_ref[g * HG + j, 0:R, :] = (_dot(p, v) * r).astype(BF)

        def cols(i, ref, rows, lo, hi):
            if i in WIDE:
                return [ref[rows, lo * LANES:hi * LANES]]
            return [ref[j, rows, :] for j in range(lo, hi)]

        def wout(c, R):
            o = jnp.concatenate([o_ref[c * OG + j, 0:R, :] for j in range(OG)], axis=1)
            w = jnp.concatenate(cols(0, wo, slice(c * OG * E, (c + 1) * OG * E), 0, ND), axis=1)
            r = _dot(o, w)
            if c > 0:
                r = r + acc_ref[0:R, :]
            if c == H // OG - 1:
                return r
            acc_ref[0:R, :] = r

        def attention(R, L, order, fillers=(), pre=None):
            ps = {}
            nxt = 0
            fillers = dict(fillers)
            for g in range(G + max(L) + 1):
                for op in order:
                    if op == "p" and g < G:
                        proj(g, R, pre)
                    if op == "q" and 0 <= g - L[0] < G:
                        ps[g - L[0]] = qk(g - L[0], R)
                    if op == "v" and 0 <= g - L[1] < G:
                        pv(g - L[1], R, ps.pop(g - L[1]))
                    if op == "w":
                        while nxt < H // OG and (nxt + 1) * OG <= (g - L[2] + 1) * HG:
                            out = wout(nxt, R)
                            nxt += 1
                    if (g - G, op) in fillers:
                        fillers.pop((g - G, op))()
            assert nxt == H // OG and not fillers
            return out

        def gate_up():
            for c in range(NF // FC):
                w = jnp.concatenate(cols(1, wg, slice(None), c * FC, (c + 1) * FC) + cols(2, wu, slice(None), c * FC, (c + 1) * FC), axis=1)
                gu = _dot(hf_ref[...], w)
                a_ref[:, c * FC * LANES:(c + 1) * FC * LANES] = (_gelu(gu[:, :FC * LANES]) * gu[:, FC * LANES:]).astype(BF)

        def down(lo, hi):
            rs = slice(lo * LANES, hi * LANES)
            return _dot(a_ref[:, rs], jnp.concatenate(cols(3, wd, rs, 0, ND), axis=1))

        def set_f(half, xr):
            xr_ref[half * SEG:(half + 1) * SEG, :] = xr
            hf_ref[half * SEG:(half + 1) * SEG, :] = _ln(xr).astype(BF)

        def out_copy(s):
            return pltpu.make_async_copy(y_v.at[seg(s), :], o_hbm.at[seg(s), :], sems.at[1])

        mem0 = mem_ref[...].astype(F32)
        h_ref[0:2 * M, :] = jnp.concatenate([mem0, mem0], axis=0).astype(BF)
        h_ref[2 * M:R1, :] = _ln(x_v[0:SEG, :].astype(F32)).astype(BF)
        for c in t_cps[0]:
            c.wait()

        def solo1(s, carry):
            out = attention(R1, LS, orderS)
            x2_v[seg(s), :] = x_v[seg(s), :].astype(F32) + out[2 * M:, :]
            h_ref[0:2 * M, :] = out[0:2 * M, :].astype(BF)
            h_ref[2 * M:R1, :] = _ln(x_v[seg(s + 1), :].astype(F32)).astype(BF)
            return carry
        lax.fori_loop(0, NS1, solo1, 0)
        for c in t_cps[1] + t_cps[2]:
            c.wait()
        set_f(0, x2_v[0:SEG, :])
        set_f(1, x2_v[SEG:2 * SEG, :])
        gate_up()
        for c in t_cps[3]:
            c.wait()
        x_cp1.start()
        x2_v[0:2 * SEG, :] = xr_ref[...] + down(0, NF)
        mem1 = h_ref[0:M, :].astype(F32)
        h_ref[0:2 * M, :] = jnp.concatenate([mem0, mem1], axis=0).astype(BF)

        def finish_attention(t, out):
            set_f(0, x2_v[seg(t - LAG), :] + out[2 * M:R1, :])
            set_f(1, x_v[seg(t), :].astype(F32) + out[R1:, :])
            h_ref[0:2 * M, :] = out[0:2 * M, :].astype(BF)

        T0 = LAG
        if LAG == 4:
            set_f(0, x2_v[2 * SEG:3 * SEG, :])
            set_f(1, x2_v[3 * SEG:4 * SEG, :])
        else:
            h_ref[2 * M:R1, :] = _ln(x2_v[0:SEG, :]).astype(BF)
            finish_attention(LAG, attention(R2, LP, orderP, pre=slice(0, SEG)))
            T0 = LAG + 1

        def steady(t, carry, pre):
            h_ref[2 * M:R1, :] = _ln(x2_v[seg(t - LAG), :]).astype(BF)
            gate_up()

            def part(lo, hi):
                def f():
                    yacc_ref[...] = (xr_ref[...] if lo == 0 else yacc_ref[...]) + down(lo, hi)
                return f
            cuts = [0] + [c for _, _, c in DP]
            fillers = {(g, op): part(cuts[i], c) for i, (g, op, c) in enumerate(DP)}
            if pre:
                out = attention(R2, LP, orderP, fillers, seg(t - LAG))
            else:
                out = attention(R2, L, order, fillers)
            finish_attention(t, out)
            h_ref[R1:R2, :] = _ln(x_v[seg(jnp.minimum(t + 1, NS - 1)), :].astype(F32)).astype(BF)
            y = yacc_ref[...] + down(cuts[-1], NF)
            x2_v[seg(t - 1), :] = y[SEG:]
            y_v[seg(t - 1 - LAG), :] = y[0:SEG].astype(BF)
            out_copy(t - 1 - LAG).start()
            return carry
        lax.fori_loop(T0, LAG + NPL, functools.partial(steady, pre=USEPRE), 0)
        x_cp1.wait()
        lax.fori_loop(LAG + NP, LAG + NST, functools.partial(steady, pre=False), 0, unroll=UN)


        def solo2(s, carry):
            out = attention(R1, LS, orderS)
            x2_v[seg(s), :] = x2_v[seg(s), :] + out[2 * M:, :]
            h_ref[0:2 * M, :] = out[0:2 * M, :].astype(BF)
            h_ref[2 * M:R1, :] = _ln(x2_v[seg(jnp.minimum(s + 1, NS - 1)), :]).astype(BF)
            return carry

        @pl.loop(0, 2)
        def _(i):
            gate_up()
            y = xr_ref[...] + down(0, NF)
            s0 = NS - 3 + i
            x2_v[seg(jnp.where(i == 0, NS - 1, NS)), :] = y[SEG:]
            y_v[seg(s0), :] = y[0:SEG].astype(BF)
            y_v[(NS - 1) * SEG:S, :] = y[SEG:].astype(BF)
            out_copy(s0).start()

            @pl.when(i == 0)
            def _():
                h_ref[2 * M:R1, :] = _ln(x2_v[(NS - 2) * SEG:(NS - 1) * SEG, :]).astype(BF)
                lax.fori_loop(NS - 2, NS, solo2, 0)
                set_f(0, x2_v[(NS - 2) * SEG:(NS - 1) * SEG, :])
                set_f(1, x2_v[(NS - 1) * SEG:S, :])
        out_copy(NS - 1).start()
        ts = list(range(T0, LAG + NPL)) + list(range(LAG + NP, LAG + NST))
        nw = (len(ts) + 1 + LAG) * SEG
        pltpu.make_async_copy(y_v.at[0:nw, :], o_hbm.at[0:nw, :], sems.at[1]).wait()

    any_spec = pl.BlockSpec(memory_space=pl.ANY)
    return pl.pallas_call(
        kern,
        out_shape=jax.ShapeDtypeStruct((S, D), BF),
        in_specs=[any_spec, pl.BlockSpec(memory_space=pltpu.VMEM)] + [any_spec] * 7,
        out_specs=any_spec,
        scratch_shapes=[
            pltpu.VMEM((S, D), BF), pltpu.VMEM((3 * NCH, CH * H, E), BF), pltpu.VMEM((3 * H, D // 2, E), U32),
            *[pltpu.VMEM((r, c * LANES) if i in WIDE else (c, r, LANES), BF)
              for i, (r, c) in enumerate(((H * E, ND), (D, NF), (D, NF), (DF, ND)))],
            pltpu.VMEM((R2, D), BF), pltpu.VMEM((NQ, R2, 3 * HG * E), BF), pltpu.VMEM((H, R2, E), BF), pltpu.VMEM((R2, D), F32),
            pltpu.VMEM((S + SEG, D), F32), pltpu.VMEM((2 * SEG, D), F32), pltpu.VMEM((2 * SEG, D), BF),
            pltpu.VMEM((2 * SEG, DF), BF), pltpu.VMEM((2 * SEG, D), F32), pltpu.VMEM((S, D), BF),
            pltpu.VMEM((NCH, NP * SEG, CH), BF), pltpu.VMEM((3 * H, NP * SEG, E), BF),
            pltpu.SemaphoreType.DMA((3,)), pltpu.SemaphoreType.DMA((3 * NCH,)), pltpu.SemaphoreType.DMA((4,)),
        ],
        compiler_params=pltpu.CompilerParams(vmem_limit_bytes=124 * 2**20, flags=flags),
    )


@functools.partial(jax.jit, static_argnames=("A_seg_len",))
def pallas_interleave_layers__memory_aug_recurrent_mem_tr__glu_gated_geglu__prompt_kernel(
    A_x, A_mem0, A_Wq, A_Wk, A_Wv, A_Wo, A_seg_len, B_x, B_w_gate, B_w_up, B_w_down
):
    del B_x
    _, S, D = A_x.shape
    _, H, E = A_Wq.shape
    M = A_mem0.shape[1]
    y = build(S, D, H, E, M, int(A_seg_len), B_w_gate.shape[1], NP=14)(
        A_x.reshape(S, D), A_mem0.reshape(M, D), A_Wq.reshape(D * H, E), A_Wk.reshape(D * H, E),
        A_Wv.reshape(D * H, E), A_Wo.reshape(H * E, D), B_w_gate, B_w_up, B_w_down)
    return y.reshape(1, S, D)
```

```python
import functools

import jax
import jax.numpy as jnp
import numpy as np
from jax import lax
from jax.experimental import pallas as pl
from jax.experimental.pallas import tpu as pltpu

BF = jnp.bfloat16
F32 = jnp.float32
U32 = jnp.uint32
LANES = 128
LAG = 2


def _ln(x):
    m = jnp.mean(x, axis=-1, keepdims=True)
    c = x - m
    v = jnp.mean(c * c, axis=-1, keepdims=True)
    return c * lax.rsqrt(v + 1e-5)


def _gelu(g):
    c0 = float(np.sqrt(2.0 / np.pi))
    return 0.5 * g * (1.0 + jnp.tanh(g * (c0 + (c0 * 0.044715) * (g * g))))


def _dot(a, b):
    return jnp.dot(a, b, preferred_element_type=F32)


def _dot_nt(a, b):
    return lax.dot_general(a, b, (((1,), (1,)), ((), ())), preferred_element_type=F32)


def build(S, D, H, E, M, SEG, DF, NP=15, HG=2, OG=4, FC=4, QH=4, NQ=4, PIPE=(1, 2, 3),
          DOWN=((0, "q", 6), (1, "q", 12), (1, "v", 18)), WO_AT=4):
    NS = S // SEG
    R1, R2 = 2 * M + SEG, 2 * M + 2 * SEG
    G = H // HG
    ND, NF = D // LANES, DF // LANES
    NCH = 8
    CH = D // NCH
    PR = NP * SEG - LAG * M
    X0 = LAG + NP + 1
    scale = float(E ** -0.5)
    assert E == LANES and H % 16 == 0 and D == 8 * E and LAG * M == 16 and (H // 8) * PR <= S

    def seg(s):
        return pl.ds(pl.multiple_of(s * SEG, SEG), SEG)

    def kern(x_hbm, mem_ref, wq_hbm, wk_hbm, wv_hbm, wo_hbm, wg_hbm, wu_hbm, wd_hbm, o_hbm,
             x_v, stage, wqkv, wo, wg, wu, wd, h_ref, qkv_ref, o_ref, acc_ref, x2_v, xr_ref, hf_ref, a_ref, yacc_ref,
             y_v, hc_ref, pad_ref, pre_ref, sems, wsems, tsems):

        def rows_copy(src, dst, lo, hi, sem):
            return pltpu.make_async_copy(src.at[lo * SEG:hi * SEG, :], dst.at[lo * SEG:hi * SEG, :], sems.at[sem])

        def out_copy(s):
            return pltpu.make_async_copy(y_v.at[seg(s), :], o_hbm.at[seg(s), :], sems.at[1])

        def chunk_copy(n, c):
            src = (wq_hbm, wk_hbm, wv_hbm)[n].at[pl.ds(pl.multiple_of(c * (CH * H), CH * H), CH * H), :]
            return pltpu.make_async_copy(src, stage.at[n * NCH + c], wsems.at[n * NCH + c])

        def start_all(cps):
            for cp in cps:
                cp.start()

        def wait_all(cps):
            for cp in cps:
                cp.wait()

        x_first, x_head, x_rest = [rows_copy(x_hbm, x_v, lo, hi, sem)
                                   for lo, hi, sem in ((LAG, X0, 0), (0, LAG, 3), (X0, NS, 2))]
        wo_cp, wg_cp, wu_cp, wd_cp = [
            [pltpu.make_async_copy(src.at[:, j * LANES:(j + 1) * LANES], dst.at[j], tsems.at[i]) for j in range(n)]
            for i, (src, dst, n) in enumerate(
                ((wo_hbm, wo, ND), (wg_hbm, wg, NF), (wu_hbm, wu, NF), (wd_hbm, wd, ND)))]

        x_first.start()
        chunk_copy(0, 0).start()
        x_first.wait()
        chunk_copy(0, 1).start()
        x_head.start()
        for s in range(NP):
            xn = _ln(x_v[(LAG + s) * SEG:(LAG + s + 1) * SEG, :].astype(F32)).astype(BF)
            k = min(SEG, PR - s * SEG)
            for c in range(NCH):
                hc_ref[c, s * SEG:s * SEG + k, :] = xn[0:k, c * CH:(c + 1) * CH]

        def octet(q):
            return [16 * (q // 2) + 2 * j + q % 2 for j in range(8)]

        def relayout(n, c, q):
            for b in range(CH // 16):
                x = pltpu.bitcast(stage[n * NCH + c, b * 16 * H:(b + 1) * 16 * H, :], U32).reshape(8, 2, H // 2, E)
                ev, od = x[:, 0, 8 * (q // 2):8 * (q // 2) + 8], x[:, 1, 8 * (q // 2):8 * (q // 2) + 8]
                w = (ev & U32(0xFFFF)) | (od << 16) if q % 2 == 0 else (ev >> 16) | (od & U32(0xFFFF0000))
                w = jnp.swapaxes(w, 0, 1)
                for j, head in enumerate(octet(q)):
                    wqkv[n * H + head, pl.ds(pl.multiple_of(c * (CH // 2) + b * 8, 8), 8), :] = w[j]

        def start_pair(n, c):
            start_all([chunk_copy(n, c), chunk_copy(n, c + 1)])

        def pre_chunk(n, c, first=False, last=False):
            i = n * NCH + c
            pltpu.make_async_copy(stage.at[i], stage.at[i], wsems.at[i]).wait()
            if first:
                pl.when(n == 0)(lambda: start_pair(0, 2))
                pl.when(n == 1)(lambda: start_all([chunk_copy(2, j) for j in range(2, NCH)]))
                pl.when(n == 2)(lambda: start_all(wg_cp + wu_cp + wd_cp))
            elif last:
                pl.when(n == 0)(lambda: start_pair(2, 0))
            else:
                @pl.when(n == 0)
                def _():
                    pl.when(2 * c + 2 < NCH)(lambda: start_pair(0, 2 * c + 2))
                    pl.when(2 * c + 2 >= NCH)(lambda: start_pair(1, 2 * c + 2 - NCH))
                pl.when(jnp.logical_and(n == 1, c == WO_AT))(lambda: start_all(wo_cp))
            r = pl.ds(pl.multiple_of(c * (CH // 2), CH // 2), CH // 2)
            relayout(n, c, 0)
            for q in range(H // 8):
                if q + 1 < H // 8:
                    relayout(n, c, q + 1)
                for h0 in range(0, 8, QH):
                    heads = octet(q)[h0:h0 + QH]
                    w = jnp.concatenate([pltpu.bitcast(wqkv[n * H + h, r, :], BF) for h in heads], axis=1)
                    blk = (slice(q * PR, (q + 1) * PR), slice(h0 * E, (h0 + QH) * E))
                    res = _dot(hc_ref[c], w)
                    if not first:
                        res = res + x2_v[blk]
                    if last:
                        for u, h in enumerate(heads):
                            pre_ref[n * H + h, 0:PR, :] = res[:, u * E:(u + 1) * E].astype(BF)
                    else:
                        x2_v[blk] = res

        @pl.loop(0, 3)
        def _(n):
            pre_chunk(n, 0, first=True)
            pl.loop(1, NCH - 1)(functools.partial(pre_chunk, n))
            pre_chunk(n, NCH - 1, last=True)

        def proj(g, R, pre, pad):
            ws = [i * H + g * HG + j for i in range(3) for j in range(HG)]
            w = jnp.concatenate([pltpu.bitcast(wqkv[n], BF) for n in ws], axis=1)
            rows = R if pre is None else R1
            qkv_ref[g % NQ, 0:rows, :] = _dot(h_ref[0:rows, :], w).astype(BF)
            for j, n in enumerate(ws):
                if pad is not None:
                    pad_ref[pad, n] = qkv_ref[g % NQ, 0:2 * M, j * E:(j + 1) * E]
                if pre is not None:
                    qkv_ref[g % NQ, R1:R2, j * E:(j + 1) * E] = pre_ref[n, pre, :]

        def qk(g, R):
            ri = lax.broadcasted_iota(jnp.int32, (R, R), 0)
            ci = lax.broadcasted_iota(jnp.int32, (R, R), 1)

            def stream(i):
                return jnp.where(i < 2 * M, (i >= M).astype(jnp.int32), (i >= R1).astype(jnp.int32))
            same = stream(ri) == stream(ci)
            valid = same & ((ri < 2 * M) | (ri >= ci))
            fill = jnp.where(same, -1e9, -jnp.inf).astype(F32)
            res = []
            for j in range(HG):
                q = qkv_ref[g % NQ, 0:R, j * E:(j + 1) * E]
                k = qkv_ref[g % NQ, 0:R, (HG + j) * E:(HG + j + 1) * E]
                s = jnp.where(valid, _dot_nt(q, k) * scale, fill)
                p = jnp.exp(s - jnp.max(s, axis=-1, keepdims=True))
                res.append((p.astype(BF), 1.0 / jnp.sum(p, axis=-1, keepdims=True)))
            return res

        def pv(g, R, res):
            for j, (p, r) in enumerate(res):
                v = qkv_ref[g % NQ, 0:R, (2 * HG + j) * E:(2 * HG + j + 1) * E]
                o_ref[g * HG + j, 0:R, :] = (_dot(p, v) * r).astype(BF)

        def wout(c, R):
            o = jnp.concatenate([o_ref[c * OG + j, 0:R, :] for j in range(OG)], axis=1)
            w = jnp.concatenate([wo[n, c * OG * E:(c + 1) * OG * E, :] for n in range(ND)], axis=1)
            r = _dot(o, w)
            if c > 0:
                r = r + acc_ref[0:R, :]
            if c < H // OG - 1:
                acc_ref[0:R, :] = r
            return r

        def attention(R, fillers=(), pre=None, pad=None):
            fillers = dict(fillers)
            probs = {}
            nxt = 0
            for g in range(G + max(PIPE) + 1):
                if g < G:
                    proj(g, R, pre, pad)
                if 0 <= g - PIPE[0] < G:
                    probs[g - PIPE[0]] = qk(g - PIPE[0], R)
                fillers.pop((g - G, "q"), lambda: None)()
                while nxt < H // OG and (nxt + 1) * OG <= (g - PIPE[2] + 1) * HG:
                    out = wout(nxt, R)
                    nxt += 1
                if 0 <= g - PIPE[1] < G:
                    pv(g - PIPE[1], R, probs.pop(g - PIPE[1]))
                fillers.pop((g - G, "v"), lambda: None)()
            assert nxt == H // OG and not fillers
            return out

        def set_ffn(half, xr):
            xr_ref[half * SEG:(half + 1) * SEG, :] = xr
            hf_ref[half * SEG:(half + 1) * SEG, :] = _ln(xr).astype(BF)

        def gate_up(extra=None):
            for c in range(NF // FC):
                if extra is not None and c == 1:
                    extra()
                tiles = range(c * FC, (c + 1) * FC)
                gu = _dot(hf_ref[...], jnp.concatenate([wg[j] for j in tiles] + [wu[j] for j in tiles], axis=1))
                a_ref[:, c * FC * LANES:(c + 1) * FC * LANES] = (
                    _gelu(gu[:, :FC * LANES]) * gu[:, FC * LANES:]).astype(BF)

        def down(lo, hi):
            rs = slice(lo * LANES, hi * LANES)
            return _dot(a_ref[:, rs], jnp.concatenate([wd[n, rs, :] for n in range(ND)], axis=1))

        x_head.wait()
        mem0 = mem_ref[...].astype(F32)
        tail = _ln(x_v[LAG * SEG + PR:(LAG + NP) * SEG, :].astype(F32))
        h_ref[0:2 * M, :] = jnp.concatenate([mem0, tail[0:M]], axis=0).astype(BF)
        h_ref[2 * M:R1, :] = _ln(x_v[0:SEG, :].astype(F32)).astype(BF)
        wait_all(wo_cp)

        @pl.loop(0, LAG)
        def _(s):
            out = attention(R1, pad=s)
            x2_v[seg(s), :] = x_v[seg(s), :].astype(F32) + out[2 * M:, :]
            h_ref[0:2 * M, :] = jnp.concatenate([out[0:M], tail[M:2 * M]], axis=0).astype(BF)
            h_ref[2 * M:R1, :] = _ln(x_v[seg(s + 1), :].astype(F32)).astype(BF)

        for n in range(3 * H):
            rows = [pad_ref[s, n].astype(F32)[M:2 * M] for s in range(LAG)]
            pre_ref[n, PR:NP * SEG, :] = jnp.concatenate(rows, axis=0).astype(BF)
        wait_all(wg_cp + wu_cp)
        set_ffn(0, x2_v[0:SEG, :])
        set_ffn(1, x2_v[SEG:2 * SEG, :])
        gate_up()
        wait_all(wd_cp)
        x_rest.start()
        x2_v[0:2 * SEG, :] = xr_ref[...] + down(0, NF)

        def finish_attention(t, out):
            set_ffn(0, x2_v[seg(t - LAG), :] + out[2 * M:R1, :])
            set_ffn(1, x_v[seg(t), :].astype(F32) + out[R1:, :])
            h_ref[0:2 * M, :] = out[0:2 * M, :].astype(BF)

        mem1 = h_ref[0:2 * M, :].astype(F32)[0:M]
        h_ref[0:2 * M, :] = jnp.concatenate([mem0, mem1], axis=0).astype(BF)
        h_ref[2 * M:R1, :] = _ln(x2_v[0:SEG, :]).astype(BF)
        finish_attention(LAG, attention(R2, pre=slice(0, SEG)))

        def dual(t, pre):
            if pre:
                pl.when(t >= LAG + 2)(lambda: out_copy(t - LAG - 2).start())
            else:
                out_copy(t - LAG - 2).start()

            def norm_a():
                h_ref[2 * M:R1, :] = _ln(x2_v[seg(t - LAG), :]).astype(BF)
            gate_up(norm_a)

            def part(lo, hi):
                def run():
                    yacc_ref[...] = (xr_ref[...] if lo == 0 else yacc_ref[...]) + down(lo, hi)
                return run
            cuts = [0] + [c for _, _, c in DOWN]
            fillers = {(g, op): part(cuts[i], c) for i, (g, op, c) in enumerate(DOWN)}
            finish_attention(t, attention(R2, fillers, pre=seg(t - LAG) if pre else None))
            h_ref[R1:R2, :] = _ln(x_v[seg(jnp.minimum(t + 1, NS - 1)), :].astype(F32)).astype(BF)
            y = yacc_ref[...] + down(cuts[-1], NF)
            x2_v[seg(t - 1), :] = y[SEG:]
            y_v[seg(t - 1 - LAG), :] = y[0:SEG].astype(BF)

        pl.loop(LAG + 1, LAG + NP)(functools.partial(dual, pre=True))
        x_rest.wait()
        pl.loop(LAG + NP, NS)(functools.partial(dual, pre=False))
        out_copy(NS - LAG - 2).start()

        @pl.loop(0, 2)
        def _(i):
            gate_up()
            y = xr_ref[...] + down(0, NF)
            x2_v[seg(jnp.where(i == 0, NS - 1, NS)), :] = y[SEG:]
            y_v[seg(NS - 3 + i), :] = y[0:SEG].astype(BF)
            y_v[(NS - 1) * SEG:S, :] = y[SEG:].astype(BF)
            out_copy(NS - 3 + i).start()

            @pl.when(i == 0)
            def _():
                h_ref[2 * M:R1, :] = _ln(x2_v[(NS - 2) * SEG:(NS - 1) * SEG, :]).astype(BF)

                @pl.loop(NS - LAG, NS)
                def _(s):
                    out = attention(R1)
                    x2_v[seg(s), :] = x2_v[seg(s), :] + out[2 * M:, :]
                    h_ref[0:2 * M, :] = out[0:2 * M, :].astype(BF)
                    h_ref[2 * M:R1, :] = _ln(x2_v[seg(jnp.minimum(s + 1, NS - 1)), :]).astype(BF)
                set_ffn(0, x2_v[(NS - 2) * SEG:(NS - 1) * SEG, :])
                set_ffn(1, x2_v[(NS - 1) * SEG:S, :])

        out_copy(NS - 1).start()
        pltpu.make_async_copy(y_v, o_hbm, sems.at[1]).wait()

    hbm = pl.BlockSpec(memory_space=pl.ANY)
    return pl.pallas_call(
        kern,
        out_shape=jax.ShapeDtypeStruct((S, D), BF),
        in_specs=[hbm, pl.BlockSpec(memory_space=pltpu.VMEM)] + [hbm] * 7,
        out_specs=hbm,
        scratch_shapes=[
            pltpu.VMEM((S, D), BF),
            pltpu.VMEM((3 * NCH, CH * H, E), BF),
            pltpu.VMEM((3 * H, D // 2, E), U32),
            pltpu.VMEM((ND, H * E, LANES), BF),
            pltpu.VMEM((NF, D, LANES), BF),
            pltpu.VMEM((NF, D, LANES), BF),
            pltpu.VMEM((ND, DF, LANES), BF),
            pltpu.VMEM((R2, D), BF),
            pltpu.VMEM((NQ, R2, 3 * HG * E), BF),
            pltpu.VMEM((H, R2, E), BF),
            pltpu.VMEM((R2, D), F32),
            pltpu.VMEM((S + SEG, D), F32),
            pltpu.VMEM((2 * SEG, D), F32),
            pltpu.VMEM((2 * SEG, D), BF),
            pltpu.VMEM((2 * SEG, DF), BF),
            pltpu.VMEM((2 * SEG, D), F32),
            pltpu.VMEM((S, D), BF),
            pltpu.VMEM((NCH, PR, CH), BF),
            pltpu.VMEM((LAG, 3 * H, 2 * M, E), BF),
            pltpu.VMEM((3 * H, NP * SEG, E), BF),
            pltpu.SemaphoreType.DMA((4,)),
            pltpu.SemaphoreType.DMA((3 * NCH,)),
            pltpu.SemaphoreType.DMA((4,)),
        ],
        compiler_params=pltpu.CompilerParams(vmem_limit_bytes=124 * 2**20),
    )


@functools.partial(jax.jit, static_argnames=("A_seg_len",))
def pallas_interleave_layers__memory_aug_recurrent_mem_tr__glu_gated_geglu__prompt_kernel(
    A_x, A_mem0, A_Wq, A_Wk, A_Wv, A_Wo, A_seg_len, B_x, B_w_gate, B_w_up, B_w_down
):
    del B_x
    _, S, D = A_x.shape
    _, H, E = A_Wq.shape
    M = A_mem0.shape[1]
    y = build(S, D, H, E, M, int(A_seg_len), B_w_gate.shape[1], QH=8)(
        A_x.reshape(S, D), A_mem0.reshape(M, D), A_Wq.reshape(D * H, E), A_Wk.reshape(D * H, E),
        A_Wv.reshape(D * H, E), A_Wo.reshape(H * E, D), B_w_gate, B_w_up, B_w_down)
    return y.reshape(1, S, D)
```

```python
import functools

import jax
import jax.numpy as jnp
import numpy as np
from jax import lax
from jax.experimental import pallas as pl
from jax.experimental.pallas import tpu as pltpu

BF = jnp.bfloat16
F32 = jnp.float32
U32 = jnp.uint32
LANES = 128
LAG = 2


def _ln(x):
    m = jnp.mean(x, axis=-1, keepdims=True)
    c = x - m
    v = jnp.mean(c * c, axis=-1, keepdims=True)
    return c * lax.rsqrt(v + 1e-5)


def _gelu(g):
    c0 = float(np.sqrt(2.0 / np.pi))
    return 0.5 * g * (1.0 + jnp.tanh(g * (c0 + (c0 * 0.044715) * (g * g))))


def _dot(a, b):
    return jnp.dot(a, b, preferred_element_type=F32)


def _dot_nt(a, b):
    return lax.dot_general(a, b, (((1,), (1,)), ((), ())), preferred_element_type=F32)


def build(S, D, H, E, M, SEG, DF, NP=16, HG=2, OG=4, FC=4, NQ=4, PIPE=(1, 2, 3),
          DOWN=((0, "q", 6), (1, "q", 12), (1, "v", 18))):
    NS = S // SEG
    R1, R2 = 2 * M + SEG, 2 * M + 2 * SEG
    G = H // HG
    ND, NF = D // LANES, DF // LANES
    NCH = 8
    CH = D // NCH
    PR = NP * SEG - LAG * M
    X0 = LAG + NP + 1
    scale = float(E ** -0.5)
    assert E == LANES and H % 16 == 0 and D == 8 * E and LAG * M == 16

    def seg(s):
        return pl.ds(pl.multiple_of(s * SEG, SEG), SEG)

    def kern(x_hbm, mem_ref, wq_hbm, wk_hbm, wv_hbm, wo_hbm, wg_hbm, wu_hbm, wd_hbm, o_hbm,
             x_v, stage, w_even, w_odd, wo, wg, wu, wd, h_ref, qkv_ref, o_ref, acc_ref, x2_v, xr_ref, hf_ref, a_ref, yacc_ref,
             y_v, hc_ref, pad_ref, pre_ref, sems, wsems, tsems):

        w_par = (w_even, w_odd)

        def rows_copy(src, dst, lo, hi, sem):
            return pltpu.make_async_copy(src.at[lo * SEG:hi * SEG, :], dst.at[lo * SEG:hi * SEG, :], sems.at[sem])

        def out_copy(s):
            return pltpu.make_async_copy(y_v.at[seg(s), :], o_hbm.at[seg(s), :], sems.at[1])

        def chunk_copy(n, c):
            src = (wq_hbm, wk_hbm, wv_hbm)[n].at[pl.ds(c * CH, CH)]
            return pltpu.make_async_copy(src, stage.at[n * NCH + c], wsems.at[n * NCH + c])

        def start_all(cps):
            for cp in cps:
                cp.start()

        def wait_all(cps):
            for cp in cps:
                cp.wait()

        x_first, x_head, x_rest = [rows_copy(x_hbm, x_v, lo, hi, sem)
                                   for lo, hi, sem in ((LAG, X0, 0), (0, LAG, 3), (X0, NS, 2))]
        wo_cp, wg_cp, wu_cp, wd_cp = [
            [pltpu.make_async_copy(src.at[:, j * LANES:(j + 1) * LANES], dst.at[j], tsems.at[i]) for j in range(n)]
            for i, (src, dst, n) in enumerate(
                ((wo_hbm, wo, ND), (wg_hbm, wg, NF), (wu_hbm, wu, NF), (wd_hbm, wd, ND)))]

        x_first.start()
        chunk_copy(0, 0).start()
        x_first.wait()
        chunk_copy(0, 1).start()
        x_head.start()
        for s in range(NP):
            xn = _ln(x_v[(LAG + s) * SEG:(LAG + s + 1) * SEG, :].astype(F32)).astype(BF)
            k = min(SEG, PR - s * SEG)
            for c in range(NCH):
                hc_ref[c, s * SEG:s * SEG + k, :] = xn[0:k, c * CH:(c + 1) * CH]

        def head_w(n, head, rows=slice(None)):
            return pltpu.bitcast(w_par[head % 2][n * (H // 2) + head // 2, rows, :], BF)

        def relayout(n, c, o, par):
            for b in range(CH // 16):
                x = stage[n * NCH + c, b * 16:(b + 1) * 16, pl.ds(pl.multiple_of(o * 16, 16), 16), :]
                x = pltpu.bitcast(x.reshape(256, E), U32).reshape(8, 2, 8, E)
                ev, od = x[:, 0], x[:, 1]
                w = (ev & U32(0xFFFF)) | (od << 16) if par == 0 else (ev >> 16) | (od & U32(0xFFFF0000))
                w = jnp.swapaxes(w, 0, 1)
                r0 = c * (CH // 2) + b * 8
                for j in range(8):
                    rows = pl.ds(r0 if isinstance(r0, int) else pl.multiple_of(r0, 8), 8)
                    w_par[par][n * (H // 2) + o * 8 + j, rows, :] = w[j]

        def wait_chunk(i):
            pltpu.make_async_copy(stage.at[i], stage.at[i], wsems.at[i]).wait()

        def start_pair(n, c):
            start_all([chunk_copy(n, c), chunk_copy(n, c + 1)])

        def q_chunk(c, first=False, last=False):
            wait_chunk(c)
            if first or last:
                start_pair(*((0, 2) if first else (2, 0)))
            else:
                pl.when(2 * c + 2 < NCH)(lambda: start_pair(0, 2 * c + 2))
                pl.when(2 * c + 2 >= NCH)(lambda: start_pair(1, 2 * c + 2 - NCH))
            r = slice(0, CH // 2) if first else slice(D // 2 - CH // 2, D // 2) if last else (
                pl.ds(pl.multiple_of(c * (CH // 2), CH // 2), CH // 2))
            relayout(0, c, 0, 0)
            for q in range(H // 8):
                if q + 1 < H // 8:
                    relayout(0, c, (q + 1) // 2, (q + 1) % 2)
                heads = [16 * (q // 2) + 2 * j + q % 2 for j in range(8)]
                res = _dot(hc_ref[c], jnp.concatenate([head_w(0, h, r) for h in heads], axis=1))
                if not first:
                    res = res + x2_v[q * PR:(q + 1) * PR, :]
                if last:
                    for u, h in enumerate(heads):
                        pre_ref[h, 0:PR, :] = res[:, u * E:(u + 1) * E].astype(BF)
                else:
                    x2_v[q * PR:(q + 1) * PR, :] = res

        q_chunk(0, first=True)
        pl.loop(1, NCH - 1)(q_chunk)
        q_chunk(NCH - 1, last=True)

        NO = H // 16
        start_all([chunk_copy(2, j) for j in range(2, NCH)])
        for c in range(NCH):
            wait_chunk(NCH + c)

        @pl.loop(0, 2 * NO)
        def _(u):
            @pl.when(u == NO - 1)
            def _():
                for c in range(NCH):
                    wait_chunk(2 * NCH + c)
                start_all(wo_cp + wg_cp)
            pl.when(u == NO)(lambda: start_all(wu_cp + wd_cp))
            n, o = 1 + u // NO, u % NO
            for par in range(2):
                for c in range(NCH):
                    relayout(n, c, o, par)
                    rows = slice(c * CH // 2, (c + 1) * CH // 2)
                    w = [pltpu.bitcast(w_par[par][n * (H // 2) + o * 8 + j, rows, :], BF) for j in range(8)]
                    res = _dot(hc_ref[c], jnp.concatenate(w, axis=1))
                    if c > 0:
                        res = res + x2_v[par * PR:(par + 1) * PR, :]
                    if c < NCH - 1:
                        x2_v[par * PR:(par + 1) * PR, :] = res
                    else:
                        for j in range(8):
                            head = n * H + 2 * (o * 8 + j) + par
                            pre_ref[head, 0:PR, :] = res[:, j * E:(j + 1) * E].astype(BF)

        def proj(g, R, pre, pad):
            ws = [i * H + g * HG + j for i in range(3) for j in range(HG)]
            w = jnp.concatenate([head_w(n // H, n % H) for n in ws], axis=1)
            rows = R if pre is None else R1
            qkv_ref[g % NQ, 0:rows, :] = _dot(h_ref[0:rows, :], w).astype(BF)
            for j, n in enumerate(ws):
                if pad is not None:
                    pad_ref[pad, n] = qkv_ref[g % NQ, 0:2 * M, j * E:(j + 1) * E]
                if pre is not None:
                    qkv_ref[g % NQ, R1:R2, j * E:(j + 1) * E] = pre_ref[n, pre, :]

        def qk(g, R):
            ri = lax.broadcasted_iota(jnp.int32, (R, R), 0)
            ci = lax.broadcasted_iota(jnp.int32, (R, R), 1)

            def stream(i):
                return jnp.where(i < 2 * M, (i >= M).astype(jnp.int32), (i >= R1).astype(jnp.int32))
            same = stream(ri) == stream(ci)
            valid = same & ((ri < 2 * M) | (ri >= ci))
            fill = jnp.where(same, -1e9, -jnp.inf).astype(F32)
            res = []
            for j in range(HG):
                q = qkv_ref[g % NQ, 0:R, j * E:(j + 1) * E]
                k = qkv_ref[g % NQ, 0:R, (HG + j) * E:(HG + j + 1) * E]
                s = jnp.where(valid, _dot_nt(q, k) * scale, fill)
                p = jnp.exp(s - jnp.max(s, axis=-1, keepdims=True))
                res.append((p.astype(BF), 1.0 / jnp.sum(p, axis=-1, keepdims=True)))
            return res

        def pv(g, R, res):
            for j, (p, r) in enumerate(res):
                v = qkv_ref[g % NQ, 0:R, (2 * HG + j) * E:(2 * HG + j + 1) * E]
                o_ref[g * HG + j, 0:R, :] = (_dot(p, v) * r).astype(BF)

        def wout(c, R):
            o = jnp.concatenate([o_ref[c * OG + j, 0:R, :] for j in range(OG)], axis=1)
            w = jnp.concatenate([wo[n, c * OG * E:(c + 1) * OG * E, :] for n in range(ND)], axis=1)
            r = _dot(o, w)
            if c > 0:
                r = r + acc_ref[0:R, :]
            if c < H // OG - 1:
                acc_ref[0:R, :] = r
            return r

        def attention(R, fillers=(), pre=None, pad=None):
            fillers = dict(fillers)
            probs = {}
            nxt = 0
            for g in range(G + max(PIPE) + 1):
                if g < G:
                    proj(g, R, pre, pad)
                if 0 <= g - PIPE[0] < G:
                    probs[g - PIPE[0]] = qk(g - PIPE[0], R)
                fillers.pop((g - G, "q"), lambda: None)()
                while nxt < H // OG and (nxt + 1) * OG <= (g - PIPE[2] + 1) * HG:
                    out = wout(nxt, R)
                    nxt += 1
                if 0 <= g - PIPE[1] < G:
                    pv(g - PIPE[1], R, probs.pop(g - PIPE[1]))
                fillers.pop((g - G, "v"), lambda: None)()
            assert nxt == H // OG and not fillers
            return out

        def set_ffn(half, xr):
            xr_ref[half * SEG:(half + 1) * SEG, :] = xr
            hf_ref[half * SEG:(half + 1) * SEG, :] = _ln(xr).astype(BF)

        def gate_up(extra=None):
            for c in range(NF // FC):
                if extra is not None and c == 1:
                    extra()
                tiles = range(c * FC, (c + 1) * FC)
                gu = _dot(hf_ref[...], jnp.concatenate([wg[j] for j in tiles] + [wu[j] for j in tiles], axis=1))
                a_ref[:, c * FC * LANES:(c + 1) * FC * LANES] = (
                    _gelu(gu[:, :FC * LANES]) * gu[:, FC * LANES:]).astype(BF)

        def down(lo, hi):
            rs = slice(lo * LANES, hi * LANES)
            return _dot(a_ref[:, rs], jnp.concatenate([wd[n, rs, :] for n in range(ND)], axis=1))

        x_head.wait()
        mem0 = mem_ref[...].astype(F32)
        tail = _ln(x_v[LAG * SEG + PR:(LAG + NP) * SEG, :].astype(F32))
        h_ref[0:2 * M, :] = jnp.concatenate([mem0, tail[0:M]], axis=0).astype(BF)
        h_ref[2 * M:R1, :] = _ln(x_v[0:SEG, :].astype(F32)).astype(BF)
        wait_all(wo_cp)

        @pl.loop(0, LAG)
        def _(s):
            out = attention(R1, pad=s)
            x2_v[seg(s), :] = x_v[seg(s), :].astype(F32) + out[2 * M:, :]
            h_ref[0:2 * M, :] = jnp.concatenate([out[0:M], tail[M:2 * M]], axis=0).astype(BF)
            h_ref[2 * M:R1, :] = _ln(x_v[seg(s + 1), :].astype(F32)).astype(BF)

        for n in range(3 * H):
            rows = [pad_ref[s, n].astype(F32)[M:2 * M] for s in range(LAG)]
            pre_ref[n, PR:NP * SEG, :] = jnp.concatenate(rows, axis=0).astype(BF)
        wait_all(wg_cp + wu_cp)
        set_ffn(0, x2_v[0:SEG, :])
        set_ffn(1, x2_v[SEG:2 * SEG, :])
        gate_up()
        wait_all(wd_cp)
        x_rest.start()
        x2_v[0:2 * SEG, :] = xr_ref[...] + down(0, NF)

        def finish_attention(t, out):
            set_ffn(0, x2_v[seg(t - LAG), :] + out[2 * M:R1, :])
            set_ffn(1, x_v[seg(t), :].astype(F32) + out[R1:, :])
            h_ref[0:2 * M, :] = out[0:2 * M, :].astype(BF)

        mem1 = h_ref[0:2 * M, :].astype(F32)[0:M]
        h_ref[0:2 * M, :] = jnp.concatenate([mem0, mem1], axis=0).astype(BF)
        h_ref[2 * M:R1, :] = _ln(x2_v[0:SEG, :]).astype(BF)
        finish_attention(LAG, attention(R2, pre=slice(0, SEG)))

        def dual(t, pre):
            if pre:
                pl.when(t >= LAG + 2)(lambda: out_copy(t - LAG - 2).start())
            else:
                out_copy(t - LAG - 2).start()

            def norm_a():
                h_ref[2 * M:R1, :] = _ln(x2_v[seg(t - LAG), :]).astype(BF)
            gate_up(norm_a)

            def part(lo, hi):
                def run():
                    yacc_ref[...] = (xr_ref[...] if lo == 0 else yacc_ref[...]) + down(lo, hi)
                return run
            cuts = [0] + [c for _, _, c in DOWN]
            fillers = {(g, op): part(cuts[i], c) for i, (g, op, c) in enumerate(DOWN)}
            finish_attention(t, attention(R2, fillers, pre=seg(t - LAG) if pre else None))
            h_ref[R1:R2, :] = _ln(x_v[seg(jnp.minimum(t + 1, NS - 1)), :].astype(F32)).astype(BF)
            y = yacc_ref[...] + down(cuts[-1], NF)
            x2_v[seg(t - 1), :] = y[SEG:]
            y_v[seg(t - 1 - LAG), :] = y[0:SEG].astype(BF)

        pl.loop(LAG + 1, LAG + NP)(functools.partial(dual, pre=True))
        x_rest.wait()
        pl.loop(LAG + NP, NS)(functools.partial(dual, pre=False))
        out_copy(NS - LAG - 2).start()

        @pl.loop(0, 2)
        def _(i):
            gate_up()
            y = xr_ref[...] + down(0, NF)
            x2_v[seg(jnp.where(i == 0, NS - 1, NS)), :] = y[SEG:]
            y_v[seg(NS - 3 + i), :] = y[0:SEG].astype(BF)
            y_v[(NS - 1) * SEG:S, :] = y[SEG:].astype(BF)
            out_copy(NS - 3 + i).start()

            @pl.when(i == 0)
            def _():
                h_ref[2 * M:R1, :] = _ln(x2_v[(NS - 2) * SEG:(NS - 1) * SEG, :]).astype(BF)

                @pl.loop(NS - LAG, NS)
                def _(s):
                    out = attention(R1)
                    x2_v[seg(s), :] = x2_v[seg(s), :] + out[2 * M:, :]
                    h_ref[0:2 * M, :] = out[0:2 * M, :].astype(BF)
                    h_ref[2 * M:R1, :] = _ln(x2_v[seg(jnp.minimum(s + 1, NS - 1)), :]).astype(BF)
                set_ffn(0, x2_v[(NS - 2) * SEG:(NS - 1) * SEG, :])
                set_ffn(1, x2_v[(NS - 1) * SEG:S, :])

        out_copy(NS - 1).start()
        pltpu.make_async_copy(y_v, o_hbm, sems.at[1]).wait()

    hbm = pl.BlockSpec(memory_space=pl.ANY)
    return pl.pallas_call(
        kern,
        out_shape=jax.ShapeDtypeStruct((S, D), BF),
        in_specs=[hbm, pl.BlockSpec(memory_space=pltpu.VMEM)] + [hbm] * 7,
        out_specs=hbm,
        scratch_shapes=[
            pltpu.VMEM((S, D), BF),
            pltpu.VMEM((3 * NCH, CH, H, E), BF),
            pltpu.VMEM((3 * H // 2, D // 2, E), U32),
            pltpu.VMEM((3 * H // 2, D // 2, E), U32),
            pltpu.VMEM((ND, H * E, LANES), BF),
            pltpu.VMEM((NF, D, LANES), BF),
            pltpu.VMEM((NF, D, LANES), BF),
            pltpu.VMEM((ND, DF, LANES), BF),
            pltpu.VMEM((R2, D), BF),
            pltpu.VMEM((NQ, R2, 3 * HG * E), BF),
            pltpu.VMEM((H, R2, E), BF),
            pltpu.VMEM((R2, D), F32),
            pltpu.VMEM((max(S + SEG, H // 8 * PR), D), F32),
            pltpu.VMEM((2 * SEG, D), F32),
            pltpu.VMEM((2 * SEG, D), BF),
            pltpu.VMEM((2 * SEG, DF), BF),
            pltpu.VMEM((2 * SEG, D), F32),
            pltpu.VMEM((S, D), BF),
            pltpu.VMEM((NCH, PR, CH), BF),
            pltpu.VMEM((LAG, 3 * H, 2 * M, E), BF),
            pltpu.VMEM((3 * H, NP * SEG, E), BF),
            pltpu.SemaphoreType.DMA((4,)),
            pltpu.SemaphoreType.DMA((3 * NCH,)),
            pltpu.SemaphoreType.DMA((4,)),
        ],
        compiler_params=pltpu.CompilerParams(vmem_limit_bytes=124 * 2**20),
    )


@functools.partial(jax.jit, static_argnames=("A_seg_len",))
def pallas_interleave_layers__memory_aug_recurrent_mem_tr__glu_gated_geglu__prompt_kernel(
    A_x, A_mem0, A_Wq, A_Wk, A_Wv, A_Wo, A_seg_len, B_x, B_w_gate, B_w_up, B_w_down
):
    del B_x
    _, S, D = A_x.shape
    _, H, E = A_Wq.shape
    M = A_mem0.shape[1]
    y = build(S, D, H, E, M, int(A_seg_len), B_w_gate.shape[1], NP=16)(
        A_x.reshape(S, D), A_mem0.reshape(M, D), A_Wq, A_Wk, A_Wv,
        A_Wo.reshape(H * E, D), B_w_gate, B_w_up, B_w_down)
    return y.reshape(1, S, D)
```

```python
import functools

import jax
import jax.numpy as jnp
import numpy as np
from jax import lax
from jax.experimental import pallas as pl
from jax.experimental.pallas import tpu as pltpu

BF = jnp.bfloat16
F32 = jnp.float32
U32 = jnp.uint32
LANES = 128
LAG = 2


def _ln(x):
    m = jnp.mean(x, axis=-1, keepdims=True)
    c = x - m
    v = jnp.mean(c * c, axis=-1, keepdims=True)
    return c * lax.rsqrt(v + 1e-5)


def _gelu(g):
    c0 = float(np.sqrt(2.0 / np.pi))
    return 0.5 * g * (1.0 + jnp.tanh(g * (c0 + (c0 * 0.044715) * (g * g))))


def _dot(a, b):
    return jnp.dot(a, b, preferred_element_type=F32)


def _dot_nt(a, b):
    return lax.dot_general(a, b, (((1,), (1,)), ((), ())), preferred_element_type=F32)


def build(S, D, H, E, M, SEG, DF, NP=16, HG=2, OG=4, FC=4, NQ=4, PIPE=(1, 2, 3),
          DOWN=((0, "q", 4), (0, "v", 8), (1, "q", 14), (1, "v", 20))):
    NS = S // SEG
    R1, R2 = 2 * M + SEG, 2 * M + 2 * SEG
    G = H // HG
    ND, NF = D // LANES, DF // LANES
    NCH = 8
    CH = D // NCH
    PR = NP * SEG - LAG * M
    X0 = LAG + NP + 1
    scale = float(E ** -0.5)
    assert E == LANES and H % 16 == 0 and D == 8 * E and LAG * M == 16

    def seg(s):
        return pl.ds(pl.multiple_of(s * SEG, SEG), SEG)

    def kern(x_hbm, mem_ref, wq_hbm, wk_hbm, wv_hbm, wo_hbm, wg_hbm, wu_hbm, wd_hbm, o_hbm,
             x_v, stage, w_even, w_odd, wo, wg, wu, wd, h_ref, qkv_ref, o_ref, acc_ref, x2_v, xr_ref, hf_ref, a_ref, yacc_ref,
             y_v, hc_ref, pad_ref, pre_ref, sems, wsems, tsems):

        w_par = (w_even, w_odd)

        def rows_copy(src, dst, lo, hi, sem):
            return pltpu.make_async_copy(src.at[lo * SEG:hi * SEG, :], dst.at[lo * SEG:hi * SEG, :], sems.at[sem])

        def out_copy(s):
            return pltpu.make_async_copy(y_v.at[seg(s), :], o_hbm.at[seg(s), :], sems.at[1])

        def chunk_copy(n, c):
            src = (wq_hbm, wk_hbm, wv_hbm)[n].at[pl.ds(c * CH, CH)]
            return pltpu.make_async_copy(src, stage.at[n * NCH + c], wsems.at[n * NCH + c])

        def start_all(cps):
            for cp in cps:
                cp.start()

        def wait_all(cps):
            for cp in cps:
                cp.wait()

        x_first, x_head, x_rest = [rows_copy(x_hbm, x_v, lo, hi, sem)
                                   for lo, hi, sem in ((LAG, X0, 0), (0, LAG, 3), (X0, NS, 2))]
        wo_cp, wg_cp, wu_cp, wd_cp = [
            [pltpu.make_async_copy(src.at[:, j * LANES:(j + 1) * LANES], dst.at[j], tsems.at[i]) for j in range(n)]
            for i, (src, dst, n) in enumerate(
                ((wo_hbm, wo, ND), (wg_hbm, wg, NF), (wu_hbm, wu, NF), (wd_hbm, wd, ND)))]

        x_first.start()
        chunk_copy(0, 0).start()
        x_first.wait()
        chunk_copy(0, 1).start()
        x_head.start()
        for s in range(NP):
            xn = _ln(x_v[(LAG + s) * SEG:(LAG + s + 1) * SEG, :].astype(F32)).astype(BF)
            k = min(SEG, PR - s * SEG)
            for c in range(NCH):
                hc_ref[c, s * SEG:s * SEG + k, :] = xn[0:k, c * CH:(c + 1) * CH]

        def head_w(n, head, rows=slice(None)):
            return pltpu.bitcast(w_par[head % 2][n * (H // 2) + head // 2, rows, :], BF)

        def relayout(n, c, o, par):
            for b in range(CH // 16):
                x = stage[n * NCH + c, b * 16:(b + 1) * 16, pl.ds(pl.multiple_of(o * 16, 16), 16), :]
                x = pltpu.bitcast(x.reshape(256, E), U32).reshape(8, 2, 8, E)
                ev, od = x[:, 0], x[:, 1]
                w = (ev & U32(0xFFFF)) | (od << 16) if par == 0 else (ev >> 16) | (od & U32(0xFFFF0000))
                w = jnp.swapaxes(w, 0, 1)
                r0 = c * (CH // 2) + b * 8
                for j in range(8):
                    rows = pl.ds(r0 if isinstance(r0, int) else pl.multiple_of(r0, 8), 8)
                    w_par[par][n * (H // 2) + o * 8 + j, rows, :] = w[j]

        def wait_chunk(i):
            pltpu.make_async_copy(stage.at[i], stage.at[i], wsems.at[i]).wait()

        def start_pair(n, c):
            start_all([chunk_copy(n, c), chunk_copy(n, c + 1)])

        def q_chunk(c, first=False, last=False):
            wait_chunk(c)
            if first or last:
                start_pair(*((0, 2) if first else (2, 0)))
            else:
                pl.when(2 * c + 2 < NCH)(lambda: start_pair(0, 2 * c + 2))
                pl.when(2 * c + 2 >= NCH)(lambda: start_pair(1, 2 * c + 2 - NCH))
            r = slice(0, CH // 2) if first else slice(D // 2 - CH // 2, D // 2) if last else (
                pl.ds(pl.multiple_of(c * (CH // 2), CH // 2), CH // 2))
            relayout(0, c, 0, 0)
            for q in range(H // 8):
                if q + 1 < H // 8:
                    relayout(0, c, (q + 1) // 2, (q + 1) % 2)
                heads = [16 * (q // 2) + 2 * j + q % 2 for j in range(8)]
                res = _dot(hc_ref[c], jnp.concatenate([head_w(0, h, r) for h in heads], axis=1))
                if not first:
                    res = res + x2_v[q * PR:(q + 1) * PR, :]
                if last:
                    for u, h in enumerate(heads):
                        pre_ref[h, 0:PR, :] = res[:, u * E:(u + 1) * E].astype(BF)
                else:
                    x2_v[q * PR:(q + 1) * PR, :] = res

        q_chunk(0, first=True)
        pl.loop(1, NCH - 1)(q_chunk)
        q_chunk(NCH - 1, last=True)

        NO = H // 16
        start_all([chunk_copy(2, j) for j in range(2, NCH)])
        for c in range(NCH):
            wait_chunk(NCH + c)

        @pl.loop(0, 2 * NO)
        def _(u):
            @pl.when(u == NO - 1)
            def _():
                for c in range(NCH):
                    wait_chunk(2 * NCH + c)
                start_all(wo_cp + wg_cp)
            pl.when(u == NO)(lambda: start_all(wu_cp + wd_cp))
            n, o = 1 + u // NO, u % NO
            for par in range(2):
                for c in range(NCH):
                    relayout(n, c, o, par)
                    rows = slice(c * CH // 2, (c + 1) * CH // 2)
                    w = [pltpu.bitcast(w_par[par][n * (H // 2) + o * 8 + j, rows, :], BF) for j in range(8)]
                    res = _dot(hc_ref[c], jnp.concatenate(w, axis=1))
                    if c > 0:
                        res = res + x2_v[par * PR:(par + 1) * PR, :]
                    if c < NCH - 1:
                        x2_v[par * PR:(par + 1) * PR, :] = res
                    else:
                        for j in range(8):
                            head = n * H + 2 * (o * 8 + j) + par
                            pre_ref[head, 0:PR, :] = res[:, j * E:(j + 1) * E].astype(BF)

        def proj(g, R, pre, pad):
            ws = [i * H + g * HG + j for i in range(3) for j in range(HG)]
            w = jnp.concatenate([head_w(n // H, n % H) for n in ws], axis=1)
            rows = R if pre is None else R1
            qkv_ref[g % NQ, 0:rows, :] = _dot(h_ref[0:rows, :], w).astype(BF)
            for j, n in enumerate(ws):
                if pad is not None:
                    pad_ref[pad, n] = qkv_ref[g % NQ, 0:2 * M, j * E:(j + 1) * E]
                if pre is not None:
                    qkv_ref[g % NQ, R1:R2, j * E:(j + 1) * E] = pre_ref[n, pre, :]

        def qk(g, R):
            ri = lax.broadcasted_iota(jnp.int32, (R, R), 0)
            ci = lax.broadcasted_iota(jnp.int32, (R, R), 1)

            def stream(i):
                return jnp.where(i < 2 * M, (i >= M).astype(jnp.int32), (i >= R1).astype(jnp.int32))
            same = stream(ri) == stream(ci)
            valid = same & ((ri < 2 * M) | (ri >= ci))
            fill = jnp.where(same, -1e9, -jnp.inf).astype(F32)
            res = []
            for j in range(HG):
                q = qkv_ref[g % NQ, 0:R, j * E:(j + 1) * E]
                k = qkv_ref[g % NQ, 0:R, (HG + j) * E:(HG + j + 1) * E]
                s = jnp.where(valid, _dot_nt(q, k) * scale, fill)
                p = jnp.exp(s - jnp.max(s, axis=-1, keepdims=True))
                res.append((p.astype(BF), 1.0 / jnp.sum(p, axis=-1, keepdims=True)))
            return res

        def pv(g, R, res):
            for j, (p, r) in enumerate(res):
                v = qkv_ref[g % NQ, 0:R, (2 * HG + j) * E:(2 * HG + j + 1) * E]
                o_ref[g * HG + j, 0:R, :] = (_dot(p, v) * r).astype(BF)

        def wout(c, R):
            o = jnp.concatenate([o_ref[c * OG + j, 0:R, :] for j in range(OG)], axis=1)
            w = jnp.concatenate([wo[n, c * OG * E:(c + 1) * OG * E, :] for n in range(ND)], axis=1)
            r = _dot(o, w)
            if c > 0:
                r = r + acc_ref[0:R, :]
            if c < H // OG - 1:
                acc_ref[0:R, :] = r
            return r

        def attention(R, fillers=(), pre=None, pad=None):
            fillers = dict(fillers)
            probs = {}
            nxt = 0
            for g in range(G + max(PIPE) + 1):
                if g < G:
                    proj(g, R, pre, pad)
                if 0 <= g - PIPE[0] < G:
                    probs[g - PIPE[0]] = qk(g - PIPE[0], R)
                fillers.pop((g - G, "q"), lambda: None)()
                while nxt < H // OG and (nxt + 1) * OG <= (g - PIPE[2] + 1) * HG:
                    out = wout(nxt, R)
                    nxt += 1
                if 0 <= g - PIPE[1] < G:
                    pv(g - PIPE[1], R, probs.pop(g - PIPE[1]))
                fillers.pop((g - G, "v"), lambda: None)()
            assert nxt == H // OG and not fillers
            return out

        def set_ffn(half, xr):
            xr_ref[half * SEG:(half + 1) * SEG, :] = xr
            hf_ref[half * SEG:(half + 1) * SEG, :] = _ln(xr).astype(BF)

        def gate_up(extra=None):
            for c in range(NF // FC):
                if extra is not None and c == 1:
                    extra()
                tiles = range(c * FC, (c + 1) * FC)
                gu = _dot(hf_ref[...], jnp.concatenate([wg[j] for j in tiles] + [wu[j] for j in tiles], axis=1))
                a_ref[:, c * FC * LANES:(c + 1) * FC * LANES] = (
                    _gelu(gu[:, :FC * LANES]) * gu[:, FC * LANES:]).astype(BF)

        def down(lo, hi):
            rs = slice(lo * LANES, hi * LANES)
            return _dot(a_ref[:, rs], jnp.concatenate([wd[n, rs, :] for n in range(ND)], axis=1))

        x_head.wait()
        mem0 = mem_ref[...].astype(F32)
        tail = _ln(x_v[LAG * SEG + PR:(LAG + NP) * SEG, :].astype(F32))
        h_ref[0:2 * M, :] = jnp.concatenate([mem0, tail[0:M]], axis=0).astype(BF)
        h_ref[2 * M:R1, :] = _ln(x_v[0:SEG, :].astype(F32)).astype(BF)
        wait_all(wo_cp)

        @pl.loop(0, LAG)
        def _(s):
            out = attention(R1, pad=s)
            x2_v[seg(s), :] = x_v[seg(s), :].astype(F32) + out[2 * M:, :]
            h_ref[0:2 * M, :] = jnp.concatenate([out[0:M], tail[M:2 * M]], axis=0).astype(BF)
            h_ref[2 * M:R1, :] = _ln(x_v[seg(s + 1), :].astype(F32)).astype(BF)

        for n in range(3 * H):
            rows = [pad_ref[s, n].astype(F32)[M:2 * M] for s in range(LAG)]
            pre_ref[n, PR:NP * SEG, :] = jnp.concatenate(rows, axis=0).astype(BF)
        wait_all(wg_cp + wu_cp)
        set_ffn(0, x2_v[0:SEG, :])
        set_ffn(1, x2_v[SEG:2 * SEG, :])
        gate_up()
        wait_all(wd_cp)
        x_rest.start()
        x2_v[0:2 * SEG, :] = xr_ref[...] + down(0, NF)

        def finish_attention(t, out):
            set_ffn(0, x2_v[seg(t - LAG), :] + out[2 * M:R1, :])
            set_ffn(1, x_v[seg(t), :].astype(F32) + out[R1:, :])
            h_ref[0:2 * M, :] = out[0:2 * M, :].astype(BF)

        mem1 = h_ref[0:2 * M, :].astype(F32)[0:M]
        h_ref[0:2 * M, :] = jnp.concatenate([mem0, mem1], axis=0).astype(BF)
        h_ref[2 * M:R1, :] = _ln(x2_v[0:SEG, :]).astype(BF)
        finish_attention(LAG, attention(R2, pre=slice(0, SEG)))

        def dual(t, pre):
            def norm_a():
                h_ref[2 * M:R1, :] = _ln(x2_v[seg(t - LAG), :]).astype(BF)
            gate_up(norm_a)

            def part(lo, hi):
                def run():
                    yacc_ref[...] = (xr_ref[...] if lo == 0 else yacc_ref[...]) + down(lo, hi)
                return run
            cuts = [0] + [c for _, _, c in DOWN]
            fillers = {(g, op): part(cuts[i], c) for i, (g, op, c) in enumerate(DOWN)}
            finish_attention(t, attention(R2, fillers, pre=seg(t - LAG) if pre else None))
            h_ref[R1:R2, :] = _ln(x_v[seg(jnp.minimum(t + 1, NS - 1)), :].astype(F32)).astype(BF)
            y = yacc_ref[...] + down(cuts[-1], NF)
            x2_v[seg(t - 1), :] = y[SEG:]
            y_v[seg(t - 1 - LAG), :] = y[0:SEG].astype(BF)

        pl.loop(LAG + 1, LAG + NP)(functools.partial(dual, pre=True))
        x_rest.wait()
        pl.loop(LAG + NP, NS)(functools.partial(dual, pre=False))
        rows_copy(y_v, o_hbm, 0, NS - LAG - 1, 1).start()

        @pl.loop(0, 2)
        def _(i):
            gate_up()
            y = xr_ref[...] + down(0, NF)
            x2_v[seg(jnp.where(i == 0, NS - 1, NS)), :] = y[SEG:]
            y_v[seg(NS - 3 + i), :] = y[0:SEG].astype(BF)
            y_v[(NS - 1) * SEG:S, :] = y[SEG:].astype(BF)
            out_copy(NS - 3 + i).start()

            @pl.when(i == 0)
            def _():
                h_ref[2 * M:R1, :] = _ln(x2_v[(NS - 2) * SEG:(NS - 1) * SEG, :]).astype(BF)

                @pl.loop(NS - LAG, NS)
                def _(s):
                    out = attention(R1)
                    x2_v[seg(s), :] = x2_v[seg(s), :] + out[2 * M:, :]
                    h_ref[0:2 * M, :] = out[0:2 * M, :].astype(BF)
                    h_ref[2 * M:R1, :] = _ln(x2_v[seg(jnp.minimum(s + 1, NS - 1)), :]).astype(BF)
                set_ffn(0, x2_v[(NS - 2) * SEG:(NS - 1) * SEG, :])
                set_ffn(1, x2_v[(NS - 1) * SEG:S, :])

        out_copy(NS - 1).start()
        pltpu.make_async_copy(y_v, o_hbm, sems.at[1]).wait()

    hbm = pl.BlockSpec(memory_space=pl.ANY)
    return pl.pallas_call(
        kern,
        out_shape=jax.ShapeDtypeStruct((S, D), BF),
        in_specs=[hbm, pl.BlockSpec(memory_space=pltpu.VMEM)] + [hbm] * 7,
        out_specs=hbm,
        scratch_shapes=[
            pltpu.VMEM((S, D), BF),
            pltpu.VMEM((3 * NCH, CH, H, E), BF),
            pltpu.VMEM((3 * H // 2, D // 2, E), U32),
            pltpu.VMEM((3 * H // 2, D // 2, E), U32),
            pltpu.VMEM((ND, H * E, LANES), BF),
            pltpu.VMEM((NF, D, LANES), BF),
            pltpu.VMEM((NF, D, LANES), BF),
            pltpu.VMEM((ND, DF, LANES), BF),
            pltpu.VMEM((R2, D), BF),
            pltpu.VMEM((NQ, R2, 3 * HG * E), BF),
            pltpu.VMEM((H, R2, E), BF),
            pltpu.VMEM((R2, D), F32),
            pltpu.VMEM((max(S + SEG, H // 8 * PR), D), F32),
            pltpu.VMEM((2 * SEG, D), F32),
            pltpu.VMEM((2 * SEG, D), BF),
            pltpu.VMEM((2 * SEG, DF), BF),
            pltpu.VMEM((2 * SEG, D), F32),
            pltpu.VMEM((S, D), BF),
            pltpu.VMEM((NCH, PR, CH), BF),
            pltpu.VMEM((LAG, 3 * H, 2 * M, E), BF),
            pltpu.VMEM((3 * H, NP * SEG, E), BF),
            pltpu.SemaphoreType.DMA((4,)),
            pltpu.SemaphoreType.DMA((3 * NCH,)),
            pltpu.SemaphoreType.DMA((4,)),
        ],
        compiler_params=pltpu.CompilerParams(vmem_limit_bytes=124 * 2**20),
    )


@functools.partial(jax.jit, static_argnames=("A_seg_len",))
def pallas_interleave_layers__memory_aug_recurrent_mem_tr__glu_gated_geglu__prompt_kernel(
    A_x, A_mem0, A_Wq, A_Wk, A_Wv, A_Wo, A_seg_len, B_x, B_w_gate, B_w_up, B_w_down
):
    del B_x
    _, S, D = A_x.shape
    _, H, E = A_Wq.shape
    M = A_mem0.shape[1]
    y = build(S, D, H, E, M, int(A_seg_len), B_w_gate.shape[1], NP=16)(
        A_x.reshape(S, D), A_mem0.reshape(M, D), A_Wq, A_Wk, A_Wv,
        A_Wo.reshape(H * E, D), B_w_gate, B_w_up, B_w_down)
    return y.reshape(1, S, D)
```

```python
import functools

import jax
import jax.numpy as jnp
import numpy as np
from jax import lax
from jax.experimental import pallas as pl
from jax.experimental.pallas import tpu as pltpu

BF = jnp.bfloat16
F32 = jnp.float32
U32 = jnp.uint32
LANES = 128
LAG = 2


def _ln(x):
    m = jnp.mean(x, axis=-1, keepdims=True)
    c = x - m
    v = jnp.mean(c * c, axis=-1, keepdims=True)
    return c * lax.rsqrt(v + 1e-5)


def _gelu(g):
    c0 = float(np.sqrt(2.0 / np.pi))
    return 0.5 * g * (1.0 + jnp.tanh(g * (c0 + (c0 * 0.044715) * (g * g))))


def _dot(a, b):
    return jnp.dot(a, b, preferred_element_type=F32)


def _dot_nt(a, b):
    return lax.dot_general(a, b, (((1,), (1,)), ((), ())), preferred_element_type=F32)


def build(S, D, H, E, M, SEG, DF, NP=16, HG=2, OG=4, FC=4, NQ=4, PIPE=(1, 2, 3), SOLO_PIPE=(1, 2, 4),
          DOWN=((0, "q", 4), (0, "v", 8), (1, "q", 14), (1, "v", 20))):
    NS = S // SEG
    R1, R2 = 2 * M + SEG, 2 * M + 2 * SEG
    G = H // HG
    ND, NF = D // LANES, DF // LANES
    NCH = 8
    CH = D // NCH
    PR = NP * SEG - LAG * M
    X0 = LAG + NP + 1
    scale = float(E ** -0.5)
    assert E == LANES and H % 16 == 0 and D == 8 * E and LAG * M == 16

    def seg(s):
        return pl.ds(pl.multiple_of(s * SEG, SEG), SEG)

    def kern(x_hbm, mem_ref, wq_hbm, wk_hbm, wv_hbm, wo_hbm, wg_hbm, wu_hbm, wd_hbm, o_hbm,
             x_v, stage, w_even, w_odd, wo, wg, wu, wd, h_ref, qkv_ref, o_ref, acc_ref, x2_v, xr_ref, hf_ref, a_ref, yacc_ref,
             y_v, hc_ref, pad_ref, pre_ref, sems, wsems, tsems):

        w_par = (w_even, w_odd)

        def rows_copy(src, dst, lo, hi, sem):
            return pltpu.make_async_copy(src.at[lo * SEG:hi * SEG, :], dst.at[lo * SEG:hi * SEG, :], sems.at[sem])

        def out_copy(s):
            return pltpu.make_async_copy(y_v.at[seg(s), :], o_hbm.at[seg(s), :], sems.at[1])

        def chunk_copy(n, c):
            src = (wq_hbm, wk_hbm, wv_hbm)[n].at[pl.ds(c * CH, CH)]
            return pltpu.make_async_copy(src, stage.at[n * NCH + c], wsems.at[n * NCH + c])

        def start_all(cps):
            for cp in cps:
                cp.start()

        def wait_all(cps):
            for cp in cps:
                cp.wait()

        x_first, x_head, x_rest = [rows_copy(x_hbm, x_v, lo, hi, sem)
                                   for lo, hi, sem in ((LAG, X0, 0), (0, LAG, 3), (X0, NS, 2))]
        wo_cp, wg_cp, wu_cp, wd_cp = [
            [pltpu.make_async_copy(src.at[:, j * LANES:(j + 1) * LANES], dst.at[j], tsems.at[i]) for j in range(n)]
            for i, (src, dst, n) in enumerate(
                ((wo_hbm, wo, ND), (wg_hbm, wg, NF), (wu_hbm, wu, NF), (wd_hbm, wd, ND)))]

        x_first.start()
        chunk_copy(0, 0).start()
        x_first.wait()
        chunk_copy(0, 1).start()
        x_head.start()
        for s in range(NP):
            xn = _ln(x_v[(LAG + s) * SEG:(LAG + s + 1) * SEG, :].astype(F32)).astype(BF)
            k = min(SEG, PR - s * SEG)
            for c in range(NCH):
                hc_ref[c, s * SEG:s * SEG + k, :] = xn[0:k, c * CH:(c + 1) * CH]

        def head_w(n, head, rows=slice(None)):
            return pltpu.bitcast(w_par[head % 2][n * (H // 2) + head // 2, rows, :], BF)

        def relayout(n, c, o, par):
            for b in range(CH // 16):
                x = stage[n * NCH + c, b * 16:(b + 1) * 16, pl.ds(pl.multiple_of(o * 16, 16), 16), :]
                x = pltpu.bitcast(x.reshape(256, E), U32).reshape(8, 2, 8, E)
                ev, od = x[:, 0], x[:, 1]
                w = (ev & np.uint32(0xFFFF)) | (od << 16) if par == 0 else (ev >> 16) | (od & np.uint32(0xFFFF0000))
                w = jnp.swapaxes(w, 0, 1)
                r0 = c * (CH // 2) + b * 8
                for j in range(8):
                    rows = pl.ds(r0 if isinstance(r0, int) else pl.multiple_of(r0, 8), 8)
                    w_par[par][n * (H // 2) + o * 8 + j, rows, :] = w[j]

        def wait_chunk(i):
            pltpu.make_async_copy(stage.at[i], stage.at[i], wsems.at[i]).wait()

        def start_pair(n, c):
            start_all([chunk_copy(n, c), chunk_copy(n, c + 1)])

        def q_chunk(c, first=False, last=False):
            wait_chunk(c)
            if first or last:
                start_pair(*((0, 2) if first else (2, 0)))
            else:
                pl.when(2 * c + 2 < NCH)(lambda: start_pair(0, 2 * c + 2))
                pl.when(2 * c + 2 >= NCH)(lambda: start_pair(1, 2 * c + 2 - NCH))
            r = slice(0, CH // 2) if first else slice(D // 2 - CH // 2, D // 2) if last else (
                pl.ds(pl.multiple_of(c * (CH // 2), CH // 2), CH // 2))
            relayout(0, c, 0, 0)
            for q in range(H // 8):
                if q + 1 < H // 8:
                    relayout(0, c, (q + 1) // 2, (q + 1) % 2)
                heads = [16 * (q // 2) + 2 * j + q % 2 for j in range(8)]
                res = _dot(hc_ref[c], jnp.concatenate([head_w(0, h, r) for h in heads], axis=1))
                if not first:
                    res = res + x2_v[q * PR:(q + 1) * PR, :]
                if last:
                    for u, h in enumerate(heads):
                        pre_ref[h, 0:PR, :] = res[:, u * E:(u + 1) * E].astype(BF)
                else:
                    x2_v[q * PR:(q + 1) * PR, :] = res

        q_chunk(0, first=True)
        pl.loop(1, NCH - 1)(q_chunk)
        q_chunk(NCH - 1, last=True)

        NO = H // 16
        start_all([chunk_copy(2, j) for j in range(2, NCH)])
        for c in range(NCH):
            wait_chunk(NCH + c)

        @pl.loop(0, 2 * NO)
        def _(u):
            @pl.when(u == NO - 1)
            def _():
                for c in range(NCH):
                    wait_chunk(2 * NCH + c)
                start_all(wo_cp + wg_cp)
            pl.when(u == NO)(lambda: start_all(wu_cp + wd_cp))
            n, o = 1 + u // NO, u % NO
            for par in range(2):
                for c in range(NCH):
                    relayout(n, c, o, par)
                    rows = slice(c * CH // 2, (c + 1) * CH // 2)
                    w = [pltpu.bitcast(w_par[par][n * (H // 2) + o * 8 + j, rows, :], BF) for j in range(8)]
                    res = _dot(hc_ref[c], jnp.concatenate(w, axis=1))
                    if c > 0:
                        res = res + x2_v[par * PR:(par + 1) * PR, :]
                    if c < NCH - 1:
                        x2_v[par * PR:(par + 1) * PR, :] = res
                    else:
                        for j in range(8):
                            head = n * H + 2 * (o * 8 + j) + par
                            pre_ref[head, 0:PR, :] = res[:, j * E:(j + 1) * E].astype(BF)

        def proj(g, R, pre, pad):
            ws = [i * H + g * HG + j for i in range(3) for j in range(HG)]
            w = jnp.concatenate([head_w(n // H, n % H) for n in ws], axis=1)
            rows = R if pre is None else R1
            qkv_ref[g % NQ, 0:rows, :] = _dot(h_ref[0:rows, :], w).astype(BF)
            for j, n in enumerate(ws):
                if pad is not None:
                    pad_ref[pad, n] = qkv_ref[g % NQ, 0:2 * M, j * E:(j + 1) * E]
                if pre is not None:
                    qkv_ref[g % NQ, R1:R2, j * E:(j + 1) * E] = pre_ref[n, pre, :]

        def qk(g, R):
            ri = lax.broadcasted_iota(jnp.int32, (R, R), 0)
            ci = lax.broadcasted_iota(jnp.int32, (R, R), 1)

            def stream(i):
                return jnp.where(i < 2 * M, (i >= M).astype(jnp.int32), (i >= R1).astype(jnp.int32))
            same = stream(ri) == stream(ci)
            valid = same & ((ri < 2 * M) | (ri >= ci))
            fill = jnp.where(same, -1e9, -jnp.inf).astype(F32)
            res = []
            for j in range(HG):
                q = qkv_ref[g % NQ, 0:R, j * E:(j + 1) * E]
                k = qkv_ref[g % NQ, 0:R, (HG + j) * E:(HG + j + 1) * E]
                s = jnp.where(valid, _dot_nt(q, k) * scale, fill)
                p = jnp.exp(s - jnp.max(s, axis=-1, keepdims=True))
                res.append((p.astype(BF), 1.0 / jnp.sum(p, axis=-1, keepdims=True)))
            return res

        def pv(g, R, res):
            for j, (p, r) in enumerate(res):
                v = qkv_ref[g % NQ, 0:R, (2 * HG + j) * E:(2 * HG + j + 1) * E]
                o_ref[g * HG + j, 0:R, :] = (_dot(p, v) * r).astype(BF)

        def wout(c, R):
            o = jnp.concatenate([o_ref[c * OG + j, 0:R, :] for j in range(OG)], axis=1)
            w = jnp.concatenate([wo[n, c * OG * E:(c + 1) * OG * E, :] for n in range(ND)], axis=1)
            r = _dot(o, w)
            if c > 0:
                r = r + acc_ref[0:R, :]
            if c < H // OG - 1:
                acc_ref[0:R, :] = r
            return r

        def attention(R, fillers=(), pre=None, pad=None):
            pipe = SOLO_PIPE if R == R1 else PIPE
            assert pipe[0] <= pipe[1] < min(pipe[2], NQ)
            fillers = dict(fillers)
            probs = {}
            nxt = 0
            for g in range(G + max(pipe) + 1):
                if g < G:
                    proj(g, R, pre, pad)
                if 0 <= g - pipe[0] < G:
                    probs[g - pipe[0]] = qk(g - pipe[0], R)
                fillers.pop((g - G, "q"), lambda: None)()
                while nxt < H // OG and (nxt + 1) * OG <= (g - pipe[2] + 1) * HG:
                    out = wout(nxt, R)
                    nxt += 1
                if 0 <= g - pipe[1] < G:
                    pv(g - pipe[1], R, probs.pop(g - pipe[1]))
                fillers.pop((g - G, "v"), lambda: None)()
            assert nxt == H // OG and not fillers
            return out

        def set_ffn(half, xr):
            xr_ref[half * SEG:(half + 1) * SEG, :] = xr
            hf_ref[half * SEG:(half + 1) * SEG, :] = _ln(xr).astype(BF)

        def gate_up(extra=None):
            for c in range(NF // FC):
                if extra is not None and c == 1:
                    extra()
                tiles = range(c * FC, (c + 1) * FC)
                gu = _dot(hf_ref[...], jnp.concatenate([wg[j] for j in tiles] + [wu[j] for j in tiles], axis=1))
                a_ref[:, c * FC * LANES:(c + 1) * FC * LANES] = (
                    _gelu(gu[:, :FC * LANES]) * gu[:, FC * LANES:]).astype(BF)

        def down(lo, hi):
            rs = slice(lo * LANES, hi * LANES)
            return _dot(a_ref[:, rs], jnp.concatenate([wd[n, rs, :] for n in range(ND)], axis=1))

        x_head.wait()
        mem0 = mem_ref[...].astype(F32)
        tail = _ln(x_v[LAG * SEG + PR:(LAG + NP) * SEG, :].astype(F32))
        h_ref[0:2 * M, :] = jnp.concatenate([mem0, tail[0:M]], axis=0).astype(BF)
        h_ref[2 * M:R1, :] = _ln(x_v[0:SEG, :].astype(F32)).astype(BF)
        wait_all(wo_cp)

        @pl.loop(0, LAG)
        def _(s):
            out = attention(R1, pad=s)
            x2_v[seg(s), :] = x_v[seg(s), :].astype(F32) + out[2 * M:, :]
            h_ref[0:2 * M, :] = jnp.concatenate([out[0:M], tail[M:2 * M]], axis=0).astype(BF)
            h_ref[2 * M:R1, :] = _ln(x_v[seg(s + 1), :].astype(F32)).astype(BF)

        for n in range(3 * H):
            rows = [pad_ref[s, n].astype(F32)[M:2 * M] for s in range(LAG)]
            pre_ref[n, PR:NP * SEG, :] = jnp.concatenate(rows, axis=0).astype(BF)
        wait_all(wg_cp + wu_cp)
        set_ffn(0, x2_v[0:SEG, :])
        set_ffn(1, x2_v[SEG:2 * SEG, :])
        gate_up()
        wait_all(wd_cp)
        x_rest.start()
        x2_v[0:2 * SEG, :] = xr_ref[...] + down(0, NF)

        def finish_attention(t, out):
            set_ffn(0, x2_v[seg(t - LAG), :] + out[2 * M:R1, :])
            set_ffn(1, x_v[seg(t), :].astype(F32) + out[R1:, :])
            h_ref[0:2 * M, :] = out[0:2 * M, :].astype(BF)

        mem1 = h_ref[0:2 * M, :].astype(F32)[0:M]
        h_ref[0:2 * M, :] = jnp.concatenate([mem0, mem1], axis=0).astype(BF)
        h_ref[2 * M:R1, :] = _ln(x2_v[0:SEG, :]).astype(BF)
        finish_attention(LAG, attention(R2, pre=slice(0, SEG)))

        def dual(t, pre):
            def norm_a():
                h_ref[2 * M:R1, :] = _ln(x2_v[seg(t - LAG), :]).astype(BF)
            gate_up(norm_a)

            def part(lo, hi):
                def run():
                    yacc_ref[...] = (xr_ref[...] if lo == 0 else yacc_ref[...]) + down(lo, hi)
                return run
            cuts = [0] + [c for _, _, c in DOWN]
            fillers = {(g, op): part(cuts[i], c) for i, (g, op, c) in enumerate(DOWN)}
            finish_attention(t, attention(R2, fillers, pre=seg(t - LAG) if pre else None))
            h_ref[R1:R2, :] = _ln(x_v[seg(jnp.minimum(t + 1, NS - 1)), :].astype(F32)).astype(BF)
            y = yacc_ref[...] + down(cuts[-1], NF)
            x2_v[seg(t - 1), :] = y[SEG:]
            y_v[seg(t - 1 - LAG), :] = y[0:SEG].astype(BF)

        pl.loop(LAG + 1, LAG + NP)(functools.partial(dual, pre=True))
        x_rest.wait()
        pl.loop(LAG + NP, NS)(functools.partial(dual, pre=False))
        rows_copy(y_v, o_hbm, 0, NS - LAG - 1, 1).start()

        @pl.loop(0, 2)
        def _(i):
            gate_up()
            y = xr_ref[...] + down(0, NF)
            x2_v[seg(jnp.where(i == 0, NS - 1, NS)), :] = y[SEG:]
            y_v[seg(NS - 3 + i), :] = y[0:SEG].astype(BF)
            y_v[(NS - 1) * SEG:S, :] = y[SEG:].astype(BF)
            out_copy(NS - 3 + i).start()

            @pl.when(i == 0)
            def _():
                h_ref[2 * M:R1, :] = _ln(x2_v[(NS - 2) * SEG:(NS - 1) * SEG, :]).astype(BF)

                @pl.loop(NS - LAG, NS)
                def _(s):
                    out = attention(R1)
                    x2_v[seg(s), :] = x2_v[seg(s), :] + out[2 * M:, :]
                    h_ref[0:2 * M, :] = out[0:2 * M, :].astype(BF)
                    h_ref[2 * M:R1, :] = _ln(x2_v[seg(jnp.minimum(s + 1, NS - 1)), :]).astype(BF)
                set_ffn(0, x2_v[(NS - 2) * SEG:(NS - 1) * SEG, :])
                set_ffn(1, x2_v[(NS - 1) * SEG:S, :])

        out_copy(NS - 1).start()
        pltpu.make_async_copy(y_v, o_hbm, sems.at[1]).wait()

    hbm = pl.BlockSpec(memory_space=pl.ANY)
    return pl.pallas_call(
        kern,
        out_shape=jax.ShapeDtypeStruct((S, D), BF),
        in_specs=[hbm, pl.BlockSpec(memory_space=pltpu.VMEM)] + [hbm] * 7,
        out_specs=hbm,
        scratch_shapes=[
            pltpu.VMEM((S, D), BF),
            pltpu.VMEM((3 * NCH, CH, H, E), BF),
            pltpu.VMEM((3 * H // 2, D // 2, E), U32),
            pltpu.VMEM((3 * H // 2, D // 2, E), U32),
            pltpu.VMEM((ND, H * E, LANES), BF),
            pltpu.VMEM((NF, D, LANES), BF),
            pltpu.VMEM((NF, D, LANES), BF),
            pltpu.VMEM((ND, DF, LANES), BF),
            pltpu.VMEM((R2, D), BF),
            pltpu.VMEM((NQ, R2, 3 * HG * E), BF),
            pltpu.VMEM((H, R2, E), BF),
            pltpu.VMEM((R2, D), F32),
            pltpu.VMEM((max(S + SEG, H // 8 * PR), D), F32),
            pltpu.VMEM((2 * SEG, D), F32),
            pltpu.VMEM((2 * SEG, D), BF),
            pltpu.VMEM((2 * SEG, DF), BF),
            pltpu.VMEM((2 * SEG, D), F32),
            pltpu.VMEM((S, D), BF),
            pltpu.VMEM((NCH, PR, CH), BF),
            pltpu.VMEM((LAG, 3 * H, 2 * M, E), BF),
            pltpu.VMEM((3 * H, NP * SEG, E), BF),
            pltpu.SemaphoreType.DMA((4,)),
            pltpu.SemaphoreType.DMA((3 * NCH,)),
            pltpu.SemaphoreType.DMA((4,)),
        ],
        compiler_params=pltpu.CompilerParams(vmem_limit_bytes=124 * 2**20),
    )


@functools.partial(jax.jit, static_argnames=("A_seg_len",))
def pallas_interleave_layers__memory_aug_recurrent_mem_tr__glu_gated_geglu__prompt_kernel(
    A_x, A_mem0, A_Wq, A_Wk, A_Wv, A_Wo, A_seg_len, B_x, B_w_gate, B_w_up, B_w_down
):
    del B_x
    _, S, D = A_x.shape
    _, H, E = A_Wq.shape
    M = A_mem0.shape[1]
    y = build(S, D, H, E, M, int(A_seg_len), B_w_gate.shape[1])(
        A_x.reshape(S, D), A_mem0.reshape(M, D), A_Wq, A_Wk, A_Wv,
        A_Wo.reshape(H * E, D), B_w_gate, B_w_up, B_w_down)
    return y.reshape(1, S, D)
```
